```python
import jax
import jax.numpy as jnp

def _softmax(x, axis=-1):
    return jax.nn.softmax(x, axis=axis)
def _gelu(x):
    return jax.nn.gelu(x, approximate=True)
def _silu(x):
    return jax.nn.silu(x)
def _sigmoid(x):
    return jax.nn.sigmoid(x)
def _layernorm(x, axis=-1, eps=1e-5):
    m = jnp.mean(x, axis=axis, keepdims=True)
    v = jnp.var(x, axis=axis, keepdims=True)
    return (x - m) / jnp.sqrt(v + eps)
def _scatter_add(tgt, idx, src, axis=0):
    return tgt.at[idx].add(src)
def _segment_sum(src, seg, n):
    return jax.ops.segment_sum(src, seg, n)
class _Rng:
    def __init__(self, key):
        self._k = key
    def _next(self):
        self._k, sub = jax.random.split(self._k)
        return sub
    def normal(self, shape):
        return jax.random.normal(self._next(), shape, dtype=jnp.bfloat16)
    def randint(self, lo, hi, shape):
        return jax.random.randint(self._next(), shape, lo, hi, dtype=jnp.int32)
    def uniform(self, shape, lo=0.0, hi=1.0):
        return jax.random.uniform(self._next(), shape, jnp.bfloat16, lo, hi)
    def permutation(self, n):
        return jax.random.permutation(self._next(), n)


kernel_name = 'recurrent_scan__sliding_local_dilated__swiglu_ffn__prompt'

def setup_inputs():
    _rng = _Rng(jax.random.key(int.from_bytes(__import__("os").urandom(4), "little")))
    _w = (lambda a: (lambda t: t.astype(jnp.bfloat16) if jnp.issubdtype(t.dtype, jnp.floating) else t)(jnp.asarray(a)))
    def _A_setup():
        B, S, D = 1, 2048, 1024
        return {
            "x": _w((lambda *s: _rng.normal(s) * 0.05)(B, S, D)),
            "wqkv": _w((lambda *s: _rng.normal(s) * 0.05)(D, 3 * D)),
            "wo": _w((lambda *s: _rng.normal(s) * 0.05)(D, D)),
        }
    _A_in = _A_setup()

    def _B_setup():
        B, S, D, F = 1, 2048, 1024, 3584
        return {
            "x": _w((lambda *s: _rng.normal(s) * 0.05)(B, S, D)),
            "w_gate": _w((lambda *s: _rng.normal(s) * 0.05)(D, F)),
            "w_up": _w((lambda *s: _rng.normal(s) * 0.05)(D, F)),
            "w_down": _w((lambda *s: _rng.normal(s) * 0.05)(F, D)),
        }
    _B_in = _B_setup()

    return {
        "A_x": _A_in["x"],
        "A_wqkv": _A_in["wqkv"],
        "A_wo": _A_in["wo"],
        "B_x": _B_in["x"],
        "B_w_gate": _B_in["w_gate"],
        "B_w_up": _B_in["w_up"],
        "B_w_down": _B_in["w_down"],
    }

def reference(A_x, A_wqkv, A_wo, B_x, B_w_gate, B_w_up, B_w_down):
    def _A_ref(x, wqkv, wo):
        B, S, D = x.shape
        H = 32; Dh = D // H
        W, dil = 8, 2
        qkv = (lambda x, *d: x.transpose(*d))((x @ wqkv).reshape(B, S, 3, H, Dh), 2, 0, 3, 1, 4)
        q, k, v = qkv[0], qkv[1], qkv[2]
        scale = Dh ** -0.5
        pos = jnp.arange(S)
        off = jnp.arange(W) * dil
        idx = pos[:, None] - off[None, :]
        mask = idx >= 0
        idx_c = jnp.where(mask, idx, 0).reshape(-1)
        kg = k[:, :, idx_c, :].reshape(B, H, S, W, Dh)
        vg = v[:, :, idx_c, :].reshape(B, H, S, W, Dh)
        logits = jnp.einsum("bhsd,bhswd->bhsw", q, kg) * scale
        logits = jnp.where(mask[None, None, :, :], logits, -1e9)
        attn = _softmax(logits, axis=-1)
        o = jnp.einsum("bhsw,bhswd->bhsd", attn, vg)
        return (lambda x, *d: x.transpose(*d))(o, 0, 2, 1, 3).reshape(B, S, D) @ wo

    def _B_ref(x, w_gate, w_up, w_down):
        g = _silu(x @ w_gate)
        u = x @ w_up
        return (g * u) @ w_down

    x = A_x
    xn = _layernorm(x, axis=-1)
    s = _A_ref(xn, A_wqkv, A_wo)
    g = _silu(_B_ref(xn, B_w_gate, B_w_up, B_w_down))
    return x + s * g
```

```python
import functools
import jax
import jax.numpy as jnp
import jax.experimental.pallas as pl
import jax.experimental.pallas.tpu as pltpu

S, D, F = 2048, 1024, 3584
H, DH, W, DIL = 32, 32, 8, 2
TM = 256
NB = S // TM
TF0 = 768
SUB = 256
NSUB = TF0 // SUB
HALO = 16
RC = 16
NC = D // 128
PS = 33
N0 = NB - 1
f32, bf16 = jnp.float32, jnp.bfloat16
FCH = [(768, 1280), (1280, 1792), (1792, 2304), (2304, 2816), (2816, 3328), (3328, 3584)]

SX, SG, SU, SD, SQ, SO, SR = 0, 8, 11, 14, 17, 23, 27
NSEM = 30


def _dot(a, b):
    return jnp.dot(a, b, preferred_element_type=f32)


def _dot_nt(a, b):
    return jax.lax.dot_general(a, b, (((1,), (1,)), ((), ())), preferred_element_type=f32)


def _silu(x):
    return x * jax.nn.sigmoid(x)


def _ln(x):
    x = x.astype(f32)
    m = jnp.mean(x, axis=-1, keepdims=True)
    xc = x - m
    var = jnp.mean(xc * xc, axis=-1, keepdims=True)
    return (xc * jax.lax.rsqrt(var + 1e-5)).astype(bf16)


def _rows(b, n=TM):
    if isinstance(b, int):
        return pl.ds(b * TM, n)
    return pl.ds(pl.multiple_of(b * TM, TM), n)


def _ds(start, size, mult):
    if isinstance(start, int):
        return pl.ds(start, size)
    return pl.ds(pl.multiple_of(start, mult), size)


def kernel(x_hbm, wqkv_hbm, wo_hbm, wg_hbm, wu_hbm, wd_hbm, o_ref,
           x_all, xn_all, acc_all, wqkv_raw, wqkv_t, wo_raw, wo_p, wg, wu, wd,
           tbuf, kbuf, vbuf, obuf, sems):
    i = pl.program_id(0)

    def cp_x(b):
        return pltpu.make_async_copy(x_hbm.at[_rows(b), :], x_all.at[_rows(b), :], sems.at[SX + b])

    def cp_g(t):
        c = _ds(t * SUB, SUB, SUB)
        return pltpu.make_async_copy(wg_hbm.at[:, c], wg.at[:, c], sems.at[SG + t])

    def cp_u(t):
        c = _ds(t * SUB, SUB, SUB)
        return pltpu.make_async_copy(wu_hbm.at[:, c], wu.at[:, c], sems.at[SU + t])

    def cp_d(t):
        c = _ds(t * SUB, SUB, SUB)
        return pltpu.make_async_copy(wd_hbm.at[c, :], wd.at[c, :], sems.at[SD + t])

    def cp_q(j):
        r = _ds((j % 2) * 512, 512, 512)
        c = _ds((j // 2) * D, D, D)
        return pltpu.make_async_copy(wqkv_hbm.at[r, c], wqkv_raw.at[r, c], sems.at[SQ + j])

    def cp_o(j):
        c = _ds(j * 256, 256, 256)
        return pltpu.make_async_copy(wo_hbm.at[:, c], wo_raw.at[:, c], sems.at[SO + j])

    def cp_rest():
        c = pl.ds(TF0, F - TF0)
        return [
            pltpu.make_async_copy(wg_hbm.at[:, c], wg.at[:, c], sems.at[SR]),
            pltpu.make_async_copy(wu_hbm.at[:, c], wu.at[:, c], sems.at[SR + 1]),
            pltpu.make_async_copy(wd_hbm.at[c, :], wd.at[c, :], sems.at[SR + 2]),
        ]

    def permute_rows(t, slot):
        for h in range(H):
            tbuf[slot, h * PS:h * PS + DH, :] = t[h * DH:(h + 1) * DH, :]
        return jnp.concatenate(
            [tbuf[slot, pl.ds(d, H, stride=PS), :] for d in range(DH)], axis=0).astype(bf16)

    @pl.when(i == 0)
    def _step0():
        cp_x(0).start()
        cp_x(1).start()
        for t in range(NSUB):
            cp_g(t).start()
            cp_u(t).start()
            cp_x(2 + t).start()
            cp_d(t).start()
        for j in range(6):
            cp_q(j).start()
            if j < 4:
                cp_o(j).start()
            if 5 + j < NB:
                cp_x(5 + j).start()
        for c in cp_rest():
            c.start()

        kbuf[:, TM:TM + HALO, :] = jnp.zeros((NC, HALO, 128), f32)
        vbuf[:, TM:TM + HALO, :] = jnp.zeros((NC, HALO, 128), f32)
        acc_all[0:2 * TM, :] = jnp.zeros((2 * TM, D), f32)
        cp_x(0).wait()
        xn_all[0:TM, :] = _ln(x_all[0:TM, :])
        cp_x(1).wait()
        xn_all[TM:2 * TM, :] = _ln(x_all[TM:2 * TM, :])

        def body(t, c):
            cols = _ds(t * SUB, SUB, SUB)
            xn = xn_all[0:2 * TM, :]
            cp_g(t).wait()
            g = _dot(xn, wg[:, cols])
            cp_u(t).wait()
            u = _dot(xn, wu[:, cols])
            h = (_silu(g) * u).astype(bf16)
            cp_x(2 + t).wait()
            cp_d(t).wait()
            acc_all[0:2 * TM, :] += _dot(h, wd[cols, :])
            xn_all[_rows(2 + t), :] = _ln(x_all[_rows(2 + t), :])
            return c
        jax.lax.fori_loop(0, NSUB, body, 0)

    @pl.when(jnp.logical_and(i >= 1, i < N0))
    def _phase0():
        b = i + 1
        j = i - 1
        cp_q(j).wait()

        @pl.when(j < 4)
        def _():
            cp_o(j).wait()

        @pl.when(b + 3 < NB)
        def _():
            cp_x(b + 3).wait()

        xn = xn_all[_rows(b), :]
        g = _dot(xn, wg[:, 0:TF0])
        u = _dot(xn, wu[:, 0:TF0])
        h = (_silu(g) * u).astype(bf16)
        acc_all[_rows(b), :] = _dot(h, wd[0:TF0, :])

        cols = _ds((j // 2) * D, D, D)
        for n in range(4):
            kb = _ds((j % 2) * 512 + n * 128, 128, 128)
            t = wqkv_raw[kb, cols].astype(f32).T
            wqkv_t[cols, kb] = permute_rows(t, n)
        jo = jnp.minimum(j, 3)
        for n in range(2):
            oc = _ds(jo * 256 + n * 128, 128, 128)
            wo_p[:, oc] = permute_rows(wo_raw[:, oc].astype(f32), 4 + n)
        bl = jnp.minimum(b + 3, NB - 1)
        xn_all[_rows(bl), :] = _ln(x_all[_rows(bl), :])

    @pl.when(i >= N0)
    def _phase1():
        b = i - N0

        @pl.when(i == N0)
        def _():
            for c in cp_rest():
                c.wait()

        kbuf[:, 0:HALO, :] = kbuf[:, TM:TM + HALO, :]
        vbuf[:, 0:HALO, :] = vbuf[:, TM:TM + HALO, :]

        xn = xn_all[_rows(b), :]
        q = _dot_nt(xn, wqkv_t[0:D, :])
        k = _dot_nt(xn, wqkv_t[D:2 * D, :])
        for c in range(NC):
            kbuf[c, HALO:HALO + TM, :] = k[:, c * 128:(c + 1) * 128]
        v = _dot_nt(xn, wqkv_t[2 * D:3 * D, :])
        for c in range(NC):
            vbuf[c, HALO:HALO + TM, :] = v[:, c * 128:(c + 1) * 128]

        scale = DH ** -0.5

        def attn(r0):
            logits = []
            for w in range(W):
                off = HALO + r0 - DIL * w
                acc = None
                for c in range(NC):
                    t = q[r0:r0 + RC, c * 128:(c + 1) * 128] * kbuf[c, off:off + RC, :]
                    acc = t if acc is None else acc + t
                acc = acc + pltpu.roll(acc, 64, 1)
                acc = acc + pltpu.roll(acc, 32, 1)
                lg = acc * scale
                if r0 < DIL * w:
                    pos = b * TM + r0 + jax.lax.broadcasted_iota(jnp.int32, (RC, 128), 0)
                    lg = jnp.where(pos >= DIL * w, lg, -1e9)
                logits.append(lg)
            mx = functools.reduce(jnp.maximum, logits)
            ps = [jnp.exp(l - mx) for l in logits]
            den = functools.reduce(lambda a, b_: a + b_, ps)
            inv = 1.0 / den
            ps = [p * inv for p in ps]
            for c in range(NC):
                acc = None
                for w in range(W):
                    off = HALO + r0 - DIL * w
                    t = ps[w] * vbuf[c, off:off + RC, :]
                    acc = t if acc is None else acc + t
                obuf[r0:r0 + RC, c * 128:(c + 1) * 128] = acc.astype(bf16)

        chunks = list(range(0, TM, RC))
        nf = len(FCH)
        acc = acc_all[_rows(b), :]
        for j, (lo_c, hi_c) in enumerate(FCH):
            g = _dot(xn, wg[:, lo_c:hi_c])
            u = _dot(xn, wu[:, lo_c:hi_c])
            h = (_silu(g) * u).astype(bf16)
            acc = acc + _dot(h, wd[lo_c:hi_c, :])
            lo = (len(chunks) * j) // (nf - 1) if j < nf - 1 else len(chunks)
            hi = (len(chunks) * (j + 1)) // (nf - 1) if j < nf - 1 else len(chunks)
            for r0 in chunks[lo:hi]:
                attn(r0)

        s = _dot(obuf[...], wo_p[...])
        x = x_all[_rows(b), :].astype(f32)
        o_ref[...] = (x + s * _silu(acc)).astype(o_ref.dtype)


@jax.jit
def pallas_recurrent_scan__sliding_local_dilated__swiglu_ffn__prompt_kernel(
    A_x, A_wqkv, A_wo, B_x, B_w_gate, B_w_up, B_w_down,
):
    x = A_x.reshape(S, D)
    out = pl.pallas_call(
        kernel,
        grid=(N0 + NB,),
        in_specs=[pl.BlockSpec(memory_space=pl.ANY)] * 6,
        out_specs=pl.BlockSpec((TM, D), lambda i: (jnp.maximum(i - N0, 0), 0)),
        out_shape=jax.ShapeDtypeStruct((S, D), bf16),
        scratch_shapes=[
            pltpu.VMEM((S, D), bf16),
            pltpu.VMEM((S, D), bf16),
            pltpu.VMEM((S, D), f32),
            pltpu.VMEM((D, 3 * D), bf16),
            pltpu.VMEM((3 * D, D), bf16),
            pltpu.VMEM((D, D), bf16),
            pltpu.VMEM((D, D), bf16),
            pltpu.VMEM((D, F), bf16),
            pltpu.VMEM((D, F), bf16),
            pltpu.VMEM((F, D), bf16),
            pltpu.VMEM((6, H * PS, 128), f32),
            pltpu.VMEM((NC, TM + HALO, 128), f32),
            pltpu.VMEM((NC, TM + HALO, 128), f32),
            pltpu.VMEM((TM, D), bf16),
            pltpu.SemaphoreType.DMA((NSEM,)),
        ],
        compiler_params=pltpu.CompilerParams(
            dimension_semantics=("arbitrary",), vmem_limit_bytes=100 * 2**20),
    )(x, A_wqkv, A_wo, B_w_gate, B_w_up, B_w_down)
    return out.reshape(1, S, D)
```

```python
import functools
import jax
import jax.numpy as jnp
import jax.experimental.pallas as pl
import jax.experimental.pallas.tpu as pltpu

S, D, F = 2048, 1024, 3584
H, DH, W, DIL = 32, 32, 8, 2
TM = 256
NB = S // TM
TF0 = 768
SUB = 256
NSUB = TF0 // SUB
HALO = 16
RC = 8
NC = D // 128
HH = H // 2
GD = 2
GPOS = 3
TB = 2 * D
DL = 10
PS = 33
N0 = NB - 1
PAD = 16
f32, bf16, u32 = jnp.float32, jnp.bfloat16, jnp.uint32
FCH = [(768, 1280), (1280, 1792), (1792, 2304), (2304, 2816), (2816, 3328), (3328, 3584)]

SX, SG, SU, SD, SQ, SO, SR = 0, 8, 11, 14, 17, 23, 27
NSEM = 30


def _dot(a, b):
    return jnp.dot(a, b, preferred_element_type=f32)


def _dot_nt(a, b):
    return jax.lax.dot_general(a, b, (((1,), (1,)), ((), ())), preferred_element_type=f32)


def _silu(x):
    h = 0.5 * x
    return h + h * jnp.tanh(h)


def _ln(x):
    m = jnp.sum(x, axis=-1, keepdims=True) * (1.0 / D)
    xc = x - m
    var = jnp.sum(xc * xc, axis=-1, keepdims=True) * (1.0 / D)
    return xc * jax.lax.rsqrt(var + 1e-5), var


def _pack2(a, b):
    return pltpu.pack_elementwise([a, b], packed_dtype=bf16)


def _unpack2(x, k):
    return pltpu.unpack_elementwise(x, index=k, packed_dtype=bf16, unpacked_dtype=f32)


def _ds(start, size, mult):
    if isinstance(start, int):
        return pl.ds(start, size)
    return pl.ds(pl.multiple_of(start, mult), size)


def _rows(b):
    return _ds(b * TM, TM, TM)


def _pack(x):
    return pltpu.bitcast(x, u32)


def _unpack(x):
    return pltpu.bitcast(x, bf16)


def kernel(x_hbm, wqkv_hbm, wo_hbm, wg_hbm, wu_hbm, wd_hbm, o_ref,
           x_all, xn_all, acc_all, wqkv_raw, wo_raw, wg, wu, wd,
           wbuf, abuf, xn_cur, sems):
    i = pl.program_id(0)
    z = jnp.minimum(i, 0)
    zvec = jnp.full((8, 128), z, jnp.int32).astype(u32)

    def delay(v, n):
        for k in range(n):
            v = (v + zvec) if k % 2 == 0 else (v ^ zvec)
        return v

    def cp_x(b):
        return pltpu.make_async_copy(x_hbm.at[_rows(b), :], x_all.at[_rows(b), :], sems.at[SX + b])

    def cp_g(t):
        c = _ds(t * SUB, SUB, SUB)
        return pltpu.make_async_copy(wg_hbm.at[:, c], wg.at[:, c], sems.at[SG + t])

    def cp_u(t):
        c = _ds(t * SUB, SUB, SUB)
        return pltpu.make_async_copy(wu_hbm.at[:, c], wu.at[:, c], sems.at[SU + t])

    def cp_d(t):
        c = _ds(t * SUB, SUB, SUB)
        return pltpu.make_async_copy(wd_hbm.at[c, :], wd.at[c, :], sems.at[SD + t])

    def cp_q(j):
        r = _ds((j % 2) * 512, 512, 512)
        c = _ds((j // 2) * D, D, D)
        return pltpu.make_async_copy(wqkv_hbm.at[r, c], wqkv_raw.at[r, c], sems.at[SQ + j])

    def cp_o(j):
        c = _ds(j * 256, 256, 256)
        return pltpu.make_async_copy(wo_hbm.at[:, c], wo_raw.at[pl.ds(0, D), c], sems.at[SO + j])

    def cp_rest():
        c = pl.ds(TF0, F - TF0)
        return [
            pltpu.make_async_copy(wg_hbm.at[:, c], wg.at[:, c], sems.at[SR]),
            pltpu.make_async_copy(wu_hbm.at[:, c], wu.at[:, c], sems.at[SR + 1]),
            pltpu.make_async_copy(wd_hbm.at[c, :], wd.at[c, :], sems.at[SR + 2]),
        ]

    def after(x, t):
        if t is None:
            return x
        return x | jnp.tile(t, (x.shape[0] // 8, x.shape[1] // 128))

    def ln_rows(start, nrows, grp, paced):
        src = x_all.at[_ds(start, nrows, 16), :]
        dst = xn_all.at[_ds(start // 2, nrows // 2, 8), :]
        t = None
        cur = src[0:grp, :]
        for r in range(0, nrows, grp):
            xw = after(_pack(cur), t)
            y0, _ = _ln(_unpack2(xw, 0))
            y1, var = _ln(_unpack2(xw, 1))
            if r + grp < nrows:
                if paced:
                    e = jnp.broadcast_to(var[grp // 2 - 8:], (8, 128))
                    x_all[S:S + 16, 0:128] = _unpack(pltpu.bitcast(e, u32))
                cur = src[r + grp:r + 2 * grp, :]
            y = _pack2(y0, y1)
            dst[r // 2:(r + grp) // 2, :] = y
            if paced:
                t = y[grp // 2 - 8:, D - 128:D] & zvec

    def load_xn(start, nrows):
        return _unpack(xn_all[_ds(start // 2, nrows // 2, 8), :])

    def scatter_rows(t, slot, m0):
        for m in range(t.shape[0] // DH):
            r = TB + (m0 + m) * PS
            wbuf[slot, r:r + DH, :] = t[m * DH:(m + 1) * DH, :]

    def gather_rows(slot, dst, t, mid=None):
        src = wbuf.at[slot + z]
        for d0 in range(0, DH, GD):
            y = jnp.concatenate(
                [src[pl.ds(TB + d, HH, stride=PS), :] for d in range(d0, d0 + GD)], axis=0)
            y = after(y, t)
            dst[d0 * HH:(d0 + GD) * HH, :] = y
            t = delay(y[GD * HH - 8:, :], DL) & zvec
            if mid is not None and d0 == DH // 2:
                mid(t)
        return t

    def load_w(r0):
        return _unpack(jnp.concatenate(
            [wbuf[c, r0:r0 + D // 2, :] for c in range(NC)], axis=1))

    def set_xn_cur(b, t):
        src = xn_all.at[_ds(b * (TM // 2), TM // 2, 8), :]
        if t is not None:
            xn_all[S // 2:S // 2 + 8, 0:128] = t
        for r in range(0, TM // 2, 8):
            y = after(src[r:r + 8, :], t)
            if t is not None:
                xn_all[S // 2:S // 2 + 8, 0:128] = y[:, 0:128]
                t = delay(y[:, D - 128:D], 2 * DL) & zvec
            xn_cur[r:r + 8, :] = y

    @pl.when(i == 0)
    @jax.named_scope('step0')
    def _step0():
        cp_x(0).start()
        cp_x(1).start()
        for t in range(NSUB):
            cp_g(t).start()
            cp_u(t).start()
            if t == 0:
                cp_x(2).start()
            cp_d(t).start()
        for j in range(6):
            cp_q(j).start()
            if j < 4:
                cp_o(j).start()
            if 3 + j < NB:
                cp_x(3 + j).start()
        for c in cp_rest():
            c.start()

        abuf[0:2 * NC, TM:TM + HALO, :] = jnp.zeros((2 * NC, HALO, 128), f32)

        def zbody(r, c):
            acc_all[_ds(r * 32, 32, 32), :] = jnp.zeros((32, D), f32)
            return c
        jax.lax.fori_loop(0, 2 * TM // 32, zbody, 0)

        def lbody(r, c):
            @pl.when(r % 2 == 0)
            def _():
                cp_x(r // 2).wait()
            ln_rows(r * 128, 128, 128, False)
            return c
        jax.lax.fori_loop(0, 4, lbody, 0)

        @jax.named_scope('s0body')
        def body(t, c):
            cols = _ds(t * SUB, SUB, SUB)
            cp_g(t).wait()
            xn = load_xn(0, 2 * TM)
            g = _dot(xn, wg[:, cols])
            cp_u(t).wait()
            u = _dot(xn, wu[:, cols])
            h = (_silu(g) * u).astype(bf16)

            @pl.when(t == 0)
            def _():
                cp_x(2).wait()
            cp_d(t).wait()
            acc_all[0:2 * TM, :] += _dot(h, wd[cols, :])
            ln_rows(2 * TM + jnp.minimum(t * 96, TM - 96), 96, 32, True)
            return c
        jax.lax.fori_loop(0, NSUB, body, 0)
        set_xn_cur(2, None)

    @pl.when(jnp.logical_and(i >= 1, i < N0))
    @jax.named_scope('phase0')
    def _phase0():
        b = i + 1
        j = i - 1
        cp_q(j).wait()

        @pl.when(j < 4)
        def _():
            cp_o(j).wait()

        @pl.when(b + 1 < NB)
        def _():
            cp_x(b + 1).wait()

        xn = _unpack(xn_cur[...])
        bn = jnp.minimum(b + 1, NB - 1)
        ln_rows(bn * TM, TM, 16, True)

        src = wqkv_raw.at[_ds((j % 2) * 512, 512, 512), _ds((j // 2) * D, D, D)]
        drows = _ds((j // 2) * (D // 2), D // 2, D // 2)
        jo = jnp.minimum(j, 3)
        osrc = wo_raw.at[:, _ds(jo * 256, 256, 256)]

        def gate_q(t):
            wqkv_raw[D:D + 16, 0:128] = _unpack(t)

        def gate_o(t):
            wo_raw[D:D + 16, 0:128] = _unpack(t)

        def ld_o(m0):
            return (osrc[m0 * DH:(m0 + 1) * DH, :], osrc[(m0 + HH) * DH:(m0 + HH + 1) * DH, :])

        t = None
        for n in range(4):
            lo = src[n * 128:(n + 1) * 128, 0:D // 2].astype(f32)
            hi = src[n * 128:(n + 1) * 128, D // 2:D].astype(f32)
            scatter_rows(_pack2(lo, hi).T, n, 0)
            t = gather_rows(n, wbuf.at[(j % 2) * 4 + n, drows], t, gate_q if n < 3 else gate_o)
        cur = ld_o(0)
        for m0 in range(HH):
            y = after(_pack2(cur[0].astype(f32), cur[1].astype(f32)), t)
            if m0 + 1 < HH:
                gate_o(y[0:8, 0:128])
                cur = ld_o(m0 + 1)
            scatter_rows(y[:, 0:128], 4, m0)
            scatter_rows(y[:, 128:256], 5, m0)
            t = delay(y[24:32, 128:256], 2 * DL) & zvec
        for n in range(2):
            t = gather_rows(4 + n, wbuf.at[jo * 2 + n, pl.ds(3 * D // 2, D // 2)], t)

        g = _dot(xn, wg[:, 0:TF0])
        u = _dot(xn, wu[:, 0:TF0])
        h = (_silu(g) * u).astype(bf16)
        acc_all[_rows(b), :] = _dot(h, wd[0:TF0, :])
        set_xn_cur(bn, pltpu.bitcast(u[TM - 8:, TF0 - 128:], u32) & zvec)

    @pl.when(i >= N0)
    @jax.named_scope('phase1')
    def _phase1():
        b = i - N0

        @pl.when(i == N0)
        def _():
            for c in cp_rest():
                c.wait()

        abuf[0:2 * NC, 0:HALO, :] = abuf[0:2 * NC, TM:TM + HALO, :]

        xn = load_xn(b * TM, TM)
        for p, base in ((1, 0), (2, NC), (0, 2 * NC)):
            y = _dot_nt(xn, load_w(p * D // 2))
            for c in range(NC):
                abuf[base + c, HALO:HALO + TM, :] = y[:, c * 128:(c + 1) * 128]

        scale = DH ** -0.5

        ab = abuf.at[pl.ds(z, 3 * NC)]

        def tok(v):
            return pltpu.bitcast(pltpu.bitcast(v, u32) & zvec, f32)

        def gate(v):
            abuf[2 * NC, 0:RC, :] = v

        def ld_q(r0):
            return [ab[2 * NC + c, HALO + r0:HALO + r0 + RC, :] for c in range(NC)]

        def ld_k(r0, w):
            off = HALO + r0 - DIL * w
            return [ab[c, off:off + RC, :] for c in range(NC)]

        def ld_v(r0, c):
            return [ab[NC + c, HALO + r0 - DIL * w:HALO + r0 - DIL * w + RC, :] for w in range(W)]

        def chain(a, bs, prev, nxt):
            ts = [x * y for x, y in zip(a, bs)]
            acc = ts[0] if prev is None else ts[0] + tok(prev)
            res = None
            for n in range(1, 8):
                acc = acc + ts[n]
                if n == GPOS and nxt is not None:
                    gate(acc)
                    res = nxt()
            return acc, res

        prev = None
        q = ld_q(0)
        cur = ld_k(0, 0)
        for r0 in range(0, TM, RC):
            logits = []
            for w in range(W):
                nxt = (lambda: ld_k(r0, w + 1)) if w < W - 1 else None
                acc, cur = chain(q, cur, prev, nxt)
                prev = acc
                acc = acc + pltpu.roll(acc, 64, 1)
                acc = acc + pltpu.roll(acc, 32, 1)
                lg = acc * scale
                if r0 < DIL * w:
                    pos = b * TM + r0 + jax.lax.broadcasted_iota(jnp.int32, (RC, 128), 0)
                    lg = jnp.where(pos >= DIL * w, lg, -1e9)
                logits.append(lg)
            mx = functools.reduce(jnp.maximum, logits)
            gate(mx)
            cur = ld_v(r0, 0)
            ps = [jnp.exp(l - mx) for l in logits]
            den = functools.reduce(lambda a, b_: a + b_, ps)
            inv = pl.reciprocal(den, approx=True)
            inv = inv * (2.0 - den * inv)
            prev = None
            for c in range(NC):
                if c < NC - 1:
                    nxt = lambda: ld_v(r0, c + 1)
                elif r0 + RC < TM:
                    nxt = lambda: (ld_q(r0 + RC), ld_k(r0 + RC, 0))
                else:
                    nxt = None
                acc, cur = chain(ps, cur, prev, nxt)
                prev = acc
                abuf[2 * NC + c, HALO + r0:HALO + r0 + RC, :] = acc * inv
            if cur is not None:
                q, cur = cur

        acc = acc_all[_rows(b), :]
        for lo_c, hi_c in FCH:
            g = _dot(xn, wg[:, lo_c:hi_c])
            u = _dot(xn, wu[:, lo_c:hi_c])
            h = (_silu(g) * u).astype(bf16)
            acc = acc + _dot(h, wd[lo_c:hi_c, :])

        o = jnp.concatenate(
            [abuf[2 * NC + c, HALO:HALO + TM, :].astype(bf16) for c in range(NC)], axis=1)
        s = _dot(o, load_w(3 * D // 2))
        x = x_all[_rows(b), :].astype(f32)
        o_ref[...] = (x + s * _silu(acc)).astype(o_ref.dtype)


@jax.jit
def pallas_recurrent_scan__sliding_local_dilated__swiglu_ffn__prompt_kernel(
    A_x, A_wqkv, A_wo, B_x, B_w_gate, B_w_up, B_w_down,
):
    x = A_x.reshape(S, D)
    out = pl.pallas_call(
        kernel,
        grid=(N0 + NB,),
        in_specs=[pl.BlockSpec(memory_space=pl.ANY)] * 6,
        out_specs=pl.BlockSpec((TM, D), lambda i: (jnp.maximum(i - N0, 0), 0)),
        out_shape=jax.ShapeDtypeStruct((S, D), bf16),
        scratch_shapes=[
            pltpu.VMEM((S + PAD, D), bf16),
            pltpu.VMEM((S // 2 + 8, D), u32),
            pltpu.VMEM((S, D), f32),
            pltpu.VMEM((D + PAD, 3 * D), bf16),
            pltpu.VMEM((D + PAD, D), bf16),
            pltpu.VMEM((D, F), bf16),
            pltpu.VMEM((D, F), bf16),
            pltpu.VMEM((F, D), bf16),
            pltpu.VMEM((NC, TB + HH * PS + 16, 128), u32),
            pltpu.VMEM((3 * NC, TM + HALO, 128), f32),
            pltpu.VMEM((TM // 2, D), u32),
            pltpu.SemaphoreType.DMA((NSEM,)),
        ],
        compiler_params=pltpu.CompilerParams(
            dimension_semantics=("arbitrary",), vmem_limit_bytes=100 * 2**20),
    )(x, A_wqkv, A_wo, B_w_gate, B_w_up, B_w_down)
    return out.reshape(1, S, D)
```

```python
import functools
import jax
import jax.numpy as jnp
import jax.experimental.pallas as pl
import jax.experimental.pallas.tpu as pltpu

S, D, F = 2048, 1024, 3584
H, DH, W, DIL = 32, 32, 8, 2
TM = 256
NB = S // TM
TF0 = 768
SUB = 256
NSUB = TF0 // SUB
HALO = 16
RC = 8
NC = D // 128
HH = H // 2
GD = 1
P0CH = [(0, 256), (256, 768)]
NPRE = 1
GPOS = 1
TB = 2 * D
DL = 6
PS = 33
N0 = NB - 1
PAD = 16
f32, bf16, u32 = jnp.float32, jnp.bfloat16, jnp.uint32
FCH = [(3328, 3584), (768, 1280), (1280, 1792), (1792, 2304), (2304, 2816), (2816, 3328)]

SX, SG, SU, SD, SQ, SO, SR = 0, 8, 11, 14, 17, 23, 27
SOUT = 30
NOP = 8
OW = D // NOP
NSEM = 32


def _dot(a, b):
    return jnp.dot(a, b, preferred_element_type=f32)


def _dot_nt(a, b):
    return jax.lax.dot_general(a, b, (((1,), (1,)), ((), ())), preferred_element_type=f32)


def _silu(x):
    h = 0.5 * x
    return h + h * jnp.tanh(h)


def _ln(x):
    m = jnp.sum(x, axis=-1, keepdims=True) * (1.0 / D)
    xc = x - m
    var = jnp.sum(xc * xc, axis=-1, keepdims=True) * (1.0 / D)
    return xc * jax.lax.rsqrt(var + 1e-5), var


def _pack2(a, b):
    return pltpu.pack_elementwise([a, b], packed_dtype=bf16)


def _unpack2(x, k):
    return pltpu.unpack_elementwise(x, index=k, packed_dtype=bf16, unpacked_dtype=f32)


def _ds(start, size, mult):
    if isinstance(start, int):
        return pl.ds(start, size)
    return pl.ds(pl.multiple_of(start, mult), size)


def _rows(b):
    return _ds(b * TM, TM, TM)


def _pack(x):
    return pltpu.bitcast(x, u32)


def _unpack(x):
    return pltpu.bitcast(x, bf16)


def kernel(x_hbm, wqkv_hbm, wo_hbm, wg_hbm, wu_hbm, wd_hbm, o_hbm,
           x_all, xn_all, acc_all, wqkv_raw, wo_raw, wg, wu, wd,
           wbuf, abuf, xn_cur, obuf, sems):
    i = pl.program_id(0)
    z = jnp.minimum(i, 0)
    zvec = jnp.full((8, 128), z, jnp.int32).astype(u32)

    def delay(v, n):
        for k in range(n):
            v = (v + zvec) if k % 2 == 0 else (v ^ zvec)
        return v

    def cp_x(b):
        return pltpu.make_async_copy(x_hbm.at[_rows(b), :], x_all.at[_rows(b), :], sems.at[SX + b])

    def cp_g(t):
        c = _ds(t * SUB, SUB, SUB)
        return pltpu.make_async_copy(wg_hbm.at[:, c], wg.at[:, c], sems.at[SG + t])

    def cp_u(t):
        c = _ds(t * SUB, SUB, SUB)
        return pltpu.make_async_copy(wu_hbm.at[:, c], wu.at[:, c], sems.at[SU + t])

    def cp_d(t):
        c = _ds(t * SUB, SUB, SUB)
        return pltpu.make_async_copy(wd_hbm.at[c, :], wd.at[c, :], sems.at[SD + t])

    def cp_q(j):
        r = _ds((j % 2) * 512, 512, 512)
        c = _ds((j // 2) * D, D, D)
        return pltpu.make_async_copy(wqkv_hbm.at[r, c], wqkv_raw.at[r, c], sems.at[SQ + j])

    def cp_o(j):
        c = _ds(j * 256, 256, 256)
        return pltpu.make_async_copy(wo_hbm.at[:, c], wo_raw.at[pl.ds(0, D), c], sems.at[SO + j])

    def cp_out(b, k=None):
        c = pl.ds(0, D) if k is None else pl.ds(k * OW, OW)
        return pltpu.make_async_copy(
            obuf.at[b % 2, :, c], o_hbm.at[_rows(b), c], sems.at[SOUT + b % 2])

    def cp_rest():
        c = pl.ds(TF0, F - TF0)
        return [
            pltpu.make_async_copy(wg_hbm.at[:, c], wg.at[:, c], sems.at[SR]),
            pltpu.make_async_copy(wu_hbm.at[:, c], wu.at[:, c], sems.at[SR + 1]),
            pltpu.make_async_copy(wd_hbm.at[c, :], wd.at[c, :], sems.at[SR + 2]),
        ]

    def after(x, t):
        if t is None:
            return x
        return x | jnp.tile(t, (x.shape[0] // 8, x.shape[1] // 128))

    def ln_rows(start, nrows, grp, paced):
        src = x_all.at[_ds(start, nrows, 16), :]
        dst = xn_all.at[_ds(start // 2, nrows // 2, 8), :]
        t = None
        cur = src[0:grp, :]
        for r in range(0, nrows, grp):
            xw = after(_pack(cur), t)
            y0, _ = _ln(_unpack2(xw, 0))
            y1, var = _ln(_unpack2(xw, 1))
            if r + grp < nrows:
                if paced:
                    e = jnp.broadcast_to(var[grp // 2 - 8:], (8, 128))
                    x_all[S:S + 16, 0:128] = _unpack(pltpu.bitcast(e, u32))
                cur = src[r + grp:r + 2 * grp, :]
            y = _pack2(y0, y1)
            dst[r // 2:(r + grp) // 2, :] = y
            if paced:
                t = y[grp // 2 - 8:, D - 128:D] & zvec

    def load_xn(start, nrows):
        return _unpack(xn_all[_ds(start // 2, nrows // 2, 8), :])

    def scatter_rows(t, slot, m0):
        for m in range(t.shape[0] // DH):
            r = TB + (m0 + m) * PS
            wbuf[slot, r:r + DH, :] = t[m * DH:(m + 1) * DH, :]

    def gather_rows(slot, dst, t, mid=None):
        src = wbuf.at[slot + z]
        for d0 in range(0, DH, GD):
            y = jnp.concatenate(
                [src[pl.ds(TB + d, HH, stride=PS), :] for d in range(d0, d0 + GD)], axis=0)
            y = after(y, t)
            dst[d0 * HH:(d0 + GD) * HH, :] = y
            t = delay(y[GD * HH - 8:, :], DL) & zvec
            if mid is not None and d0 == DH // 2:
                mid(t)
        return t

    def load_w(r0):
        return _unpack(jnp.concatenate(
            [wbuf[c, r0:r0 + D // 2, :] for c in range(NC)], axis=1))

    def set_xn_cur(b, t):
        src = xn_all.at[_ds(b * (TM // 2), TM // 2, 8), :]
        if t is not None:
            xn_all[S // 2:S // 2 + 8, 0:128] = t
        for r in range(0, TM // 2, 8):
            y = after(src[r:r + 8, :], t)
            if t is not None:
                xn_all[S // 2:S // 2 + 8, 0:128] = y[:, 0:128]
                t = delay(y[:, D - 128:D], 2 * DL) & zvec
            xn_cur[r:r + 8, :] = y

    @pl.when(i == 0)
    @jax.named_scope('step0')
    def _step0():
        cp_x(0).start()
        cp_x(1).start()
        for t in range(NSUB):
            cp_g(t).start()
            cp_u(t).start()
            if t == 0:
                cp_x(2).start()
            cp_d(t).start()
        for j in range(6):
            cp_q(j).start()
            if j < 4:
                cp_o(j).start()
            if 3 + j < NB:
                cp_x(3 + j).start()
        for c in cp_rest():
            c.start()

        abuf[0:2 * NC, TM:TM + HALO, :] = jnp.zeros((2 * NC, HALO, 128), f32)

        def zbody(r, c):
            acc_all[_ds(r * 32, 32, 32), :] = jnp.zeros((32, D), f32)
            return c
        jax.lax.fori_loop(0, 2 * TM // 32, zbody, 0)

        def lbody(r, c):
            @pl.when(r % 2 == 0)
            def _():
                cp_x(r // 2).wait()
            ln_rows(r * 128, 128, 128, False)
            return c
        jax.lax.fori_loop(0, 4, lbody, 0)

        @jax.named_scope('s0body')
        def body(t, c):
            cols = _ds(t * SUB, SUB, SUB)
            cp_g(t).wait()
            xn = load_xn(0, 2 * TM)
            g = _dot(xn, wg[:, cols])
            cp_u(t).wait()
            u = _dot(xn, wu[:, cols])
            h = (_silu(g) * u).astype(bf16)

            @pl.when(t == 0)
            def _():
                cp_x(2).wait()
            cp_d(t).wait()
            acc_all[0:2 * TM, :] += _dot(h, wd[cols, :])
            ln_rows(2 * TM + jnp.minimum(t * 96, TM - 96), 96, 32, True)
            return c
        jax.lax.fori_loop(0, NSUB, body, 0)
        set_xn_cur(2, None)

    @pl.when(jnp.logical_and(i >= 1, i < N0))
    @jax.named_scope('phase0')
    def _phase0():
        b = i + 1
        j = i - 1
        cp_q(j).wait()

        @pl.when(j < 4)
        def _():
            cp_o(j).wait()

        @pl.when(b + 1 < NB)
        def _():
            cp_x(b + 1).wait()

        xn = _unpack(xn_cur[...])
        bn = jnp.minimum(b + 1, NB - 1)
        ln_rows(bn * TM, TM, 16, True)

        src = wqkv_raw.at[_ds((j % 2) * 512, 512, 512), _ds((j // 2) * D, D, D)]
        drows = _ds((j // 2) * (D // 2), D // 2, D // 2)
        jo = jnp.minimum(j, 3)
        osrc = wo_raw.at[:, _ds(jo * 256, 256, 256)]

        def gate_q(t):
            wqkv_raw[D:D + 16, 0:128] = _unpack(t)

        def gate_o(t):
            wo_raw[D:D + 16, 0:128] = _unpack(t)

        def ld_o(m0):
            return (osrc[m0 * DH:(m0 + 1) * DH, :], osrc[(m0 + HH) * DH:(m0 + HH + 1) * DH, :])

        t = None
        for n in range(4):
            lo = src[n * 128:(n + 1) * 128, 0:D // 2].astype(f32)
            hi = src[n * 128:(n + 1) * 128, D // 2:D].astype(f32)
            scatter_rows(_pack2(lo, hi).T, n, 0)
            t = gather_rows(n, wbuf.at[(j % 2) * 4 + n, drows], t, gate_q if n < 3 else gate_o)
        cur = ld_o(0)
        for m0 in range(HH):
            y = after(_pack2(cur[0].astype(f32), cur[1].astype(f32)), t)
            if m0 + 1 < HH:
                gate_o(y[0:8, 0:128])
                cur = ld_o(m0 + 1)
            scatter_rows(y[:, 0:128], 4, m0)
            scatter_rows(y[:, 128:256], 5, m0)
            t = delay(y[24:32, 128:256], 2 * DL) & zvec
        for n in range(2):
            t = gather_rows(4 + n, wbuf.at[jo * 2 + n, pl.ds(3 * D // 2, D // 2)], t)

        acc = None
        for lo_c, hi_c in P0CH:
            g = _dot(xn, wg[:, lo_c:hi_c])
            u = _dot(xn, wu[:, lo_c:hi_c])
            h = (_silu(g) * u).astype(bf16)
            d = _dot(h, wd[lo_c:hi_c, :])
            acc = d if acc is None else acc + d
        acc_all[_rows(b), :] = acc
        set_xn_cur(bn, pltpu.bitcast(u[TM - 8:, u.shape[1] - 128:], u32) & zvec)

    @pl.when(i >= N0)
    @jax.named_scope('phase1')
    def _phase1():
        b = i - N0

        @pl.when(i == N0)
        def _():
            for c in cp_rest():
                c.wait()

        @pl.when(b >= 2)
        def _():
            cp_out(b - 2).wait()

        abuf[0:2 * NC, 0:HALO, :] = abuf[0:2 * NC, TM:TM + HALO, :]

        xn = load_xn(b * TM, TM)

        def ffn(acc, lo_c, hi_c):
            g = _dot(xn, wg[:, lo_c:hi_c])
            u = _dot(xn, wu[:, lo_c:hi_c])
            h = (_silu(g) * u).astype(bf16)
            return acc + _dot(h, wd[lo_c:hi_c, :])

        acc = acc_all[_rows(b), :]
        for ch in FCH[:NPRE]:
            acc = ffn(acc, *ch)
        facc = acc
        for p, base in ((1, 0), (2, NC), (0, 2 * NC)):
            y = _dot_nt(xn, load_w(p * D // 2))
            for c in range(NC):
                abuf[base + c, HALO:HALO + TM, :] = y[:, c * 128:(c + 1) * 128]

        scale = DH ** -0.5

        ab = abuf.at[pl.ds(z, 3 * NC)]

        def tok(v):
            return pltpu.bitcast(pltpu.bitcast(v, u32) & zvec, f32)

        def gate(v):
            abuf[2 * NC, 0:RC, :] = v

        def ld_q(r0):
            return [ab[2 * NC + c, HALO + r0:HALO + r0 + RC, :] for c in range(NC)]

        def ld_k(r0, w):
            off = HALO + r0 - DIL * w
            return [ab[c, off:off + RC, :] for c in range(NC)]

        def ld_v(r0, c):
            return [ab[NC + c, HALO + r0 - DIL * w:HALO + r0 - DIL * w + RC, :] for w in range(W)]

        def chain(a, bs, prev, nxt):
            ts = [x * y for x, y in zip(a, bs)]
            acc = ts[0] if prev is None else ts[0] + tok(prev)
            res = None
            for n in range(1, 8):
                acc = acc + ts[n]
                if n == GPOS and nxt is not None:
                    gate(acc)
                    res = nxt()
            return acc, res

        prev = None
        q = ld_q(0)
        cur = ld_k(0, 0)
        for r0 in range(0, TM, RC):
            logits = []
            for w in range(W):
                nxt = (lambda: ld_k(r0, w + 1)) if w < W - 1 else None
                acc, cur = chain(q, cur, prev, nxt)
                prev = acc
                acc = acc + pltpu.roll(acc, 64, 1)
                acc = acc + pltpu.roll(acc, 32, 1)
                lg = acc * scale
                if r0 < DIL * w:
                    pos = b * TM + r0 + jax.lax.broadcasted_iota(jnp.int32, (RC, 128), 0)
                    lg = jnp.where(pos >= DIL * w, lg, -1e9)
                logits.append(lg)
            mx = functools.reduce(jnp.maximum, logits)
            gate(mx)
            cur = ld_v(r0, 0)
            ps = [jnp.exp(l - mx) for l in logits]
            den = functools.reduce(lambda a, b_: a + b_, ps)
            inv = pl.reciprocal(den, approx=True)
            inv = inv * (2.0 - den * inv)
            prev = None
            for c in range(NC):
                if c < NC - 1:
                    nxt = lambda: ld_v(r0, c + 1)
                elif r0 + RC < TM:
                    nxt = lambda: (ld_q(r0 + RC), ld_k(r0 + RC, 0))
                else:
                    nxt = None
                acc, cur = chain(ps, cur, prev, nxt)
                prev = acc
                abuf[2 * NC + c, HALO + r0:HALO + r0 + RC, :] = acc * inv
            if cur is not None:
                q, cur = cur

        acc = facc
        for ch in FCH[NPRE:]:
            acc = ffn(acc, *ch)

        o = jnp.concatenate(
            [abuf[2 * NC + c, HALO:HALO + TM, :].astype(bf16) for c in range(NC)], axis=1)
        s = _dot(o, load_w(3 * D // 2))
        ob = obuf.at[b % 2]
        for k in range(NOP):
            c = slice(k * OW, (k + 1) * OW)
            x = x_all[_rows(b), c].astype(f32)
            ob[:, c] = (x + s[:, c] * _silu(acc[:, c])).astype(bf16)
            cp_out(b, k).start()

        @pl.when(b == NB - 1)
        def _():
            cp_out(b - 1).wait()
            cp_out(b).wait()


@jax.jit
def pallas_recurrent_scan__sliding_local_dilated__swiglu_ffn__prompt_kernel(
    A_x, A_wqkv, A_wo, B_x, B_w_gate, B_w_up, B_w_down,
):
    x = A_x.reshape(S, D)
    out = pl.pallas_call(
        kernel,
        grid=(N0 + NB,),
        in_specs=[pl.BlockSpec(memory_space=pl.ANY)] * 6,
        out_specs=pl.BlockSpec(memory_space=pl.ANY),
        out_shape=jax.ShapeDtypeStruct((S, D), bf16),
        scratch_shapes=[
            pltpu.VMEM((S + PAD, D), bf16),
            pltpu.VMEM((S // 2 + 8, D), u32),
            pltpu.VMEM((S, D), f32),
            pltpu.VMEM((D + PAD, 3 * D), bf16),
            pltpu.VMEM((D + PAD, D), bf16),
            pltpu.VMEM((D, F), bf16),
            pltpu.VMEM((D, F), bf16),
            pltpu.VMEM((F, D), bf16),
            pltpu.VMEM((NC, TB + HH * PS + 16, 128), u32),
            pltpu.VMEM((3 * NC, TM + HALO, 128), f32),
            pltpu.VMEM((TM // 2, D), u32),
            pltpu.VMEM((2, TM, D), bf16),
            pltpu.SemaphoreType.DMA((NSEM,)),
        ],
        compiler_params=pltpu.CompilerParams(
            dimension_semantics=("arbitrary",), vmem_limit_bytes=100 * 2**20,
            disable_bounds_checks=True, disable_semaphore_checks=True),
    )(x, A_wqkv, A_wo, B_w_gate, B_w_up, B_w_down)
    return out.reshape(1, S, D)
```

```python
import functools
import jax
import jax.numpy as jnp
import jax.experimental.pallas as pl
import jax.experimental.pallas.tpu as pltpu

S, D, F = 2048, 1024, 3584
H, DH, W, DIL = 32, 32, 8, 2
TM = 256
NB = S // TM
TF0 = 768
SUB = 256
NSUB = TF0 // SUB
HALO = 16
RC = 8
NC = D // 128
HH = H // 2
GD = 1
R3SPLIT = [(0, 4), (4, 16)]
P0CH = [(0, 256), (256, 768)]
NPRE = 1
GPOS = 1
TB = 2 * D
DL = 6
PS = 33
N0 = NB - 1
PAD = 16
f32, bf16, u32 = jnp.float32, jnp.bfloat16, jnp.uint32
FCH = [(3328, 3584), (768, 1280), (1280, 1792), (1792, 2304), (2304, 2816), (2816, 3328)]

SX, SG, SU, SD, SQ, SO, SR = 0, 8, 11, 14, 17, 23, 27
SOUT = 30
NOP = 8
OW = D // NOP
NSEM = 32


def _dot(a, b):
    return jnp.dot(a, b, preferred_element_type=f32)


def _dot_nt(a, b):
    return jax.lax.dot_general(a, b, (((1,), (1,)), ((), ())), preferred_element_type=f32)


def _silu(x):
    h = 0.5 * x
    return h + h * jnp.tanh(h)


def _ln(x):
    m = jnp.sum(x, axis=-1, keepdims=True) * (1.0 / D)
    xc = x - m
    var = jnp.sum(xc * xc, axis=-1, keepdims=True) * (1.0 / D)
    return xc * jax.lax.rsqrt(var + 1e-5), var


def _pack2(a, b):
    return pltpu.pack_elementwise([a, b], packed_dtype=bf16)


def _unpack2(x, k):
    return pltpu.unpack_elementwise(x, index=k, packed_dtype=bf16, unpacked_dtype=f32)


def _ds(start, size, mult):
    if isinstance(start, int):
        return pl.ds(start, size)
    return pl.ds(pl.multiple_of(start, mult), size)


def _rows(b):
    return _ds(b * TM, TM, TM)


def _pack(x):
    return pltpu.bitcast(x, u32)


def _unpack(x):
    return pltpu.bitcast(x, bf16)


def kernel(x_hbm, wqkv_hbm, wo_hbm, wg_hbm, wu_hbm, wd_hbm, o_hbm,
           x_all, xn_all, acc_all, wqkv_raw, wo_raw, wg, wu, wd,
           wbuf, abuf, xn_cur, obuf, sems):
    i = pl.program_id(0)
    z = jnp.minimum(i, 0)
    zvec = jnp.full((8, 128), z, jnp.int32).astype(u32)

    def delay(v, n):
        for k in range(n):
            v = (v + zvec) if k % 2 == 0 else (v ^ zvec)
        return v

    def cp_x(b):
        return pltpu.make_async_copy(x_hbm.at[_rows(b), :], x_all.at[_rows(b), :], sems.at[SX + b])

    def cp_g(t):
        c = _ds(t * SUB, SUB, SUB)
        return pltpu.make_async_copy(wg_hbm.at[:, c], wg.at[:, c], sems.at[SG + t])

    def cp_u(t):
        c = _ds(t * SUB, SUB, SUB)
        return pltpu.make_async_copy(wu_hbm.at[:, c], wu.at[:, c], sems.at[SU + t])

    def cp_d(t):
        c = _ds(t * SUB, SUB, SUB)
        return pltpu.make_async_copy(wd_hbm.at[c, :], wd.at[c, :], sems.at[SD + t])

    def cp_q(j):
        r = _ds((j & 1) * 512, 512, 512)
        c = _ds((j >> 1) * D, D, D)
        return pltpu.make_async_copy(wqkv_hbm.at[r, c], wqkv_raw.at[r, c], sems.at[SQ + j])

    def cp_o(j):
        c = _ds(j * 256, 256, 256)
        return pltpu.make_async_copy(wo_hbm.at[:, c], wo_raw.at[pl.ds(0, D), c], sems.at[SO + j])

    def cp_out(b, k=None):
        c = pl.ds(0, D) if k is None else pl.ds(k * OW, OW)
        return pltpu.make_async_copy(
            obuf.at[b & 1, :, c], o_hbm.at[_rows(b), c], sems.at[SOUT + (b & 1)])

    def cp_rest():
        c = pl.ds(TF0, F - TF0)
        return [
            pltpu.make_async_copy(wg_hbm.at[:, c], wg.at[:, c], sems.at[SR]),
            pltpu.make_async_copy(wu_hbm.at[:, c], wu.at[:, c], sems.at[SR + 1]),
            pltpu.make_async_copy(wd_hbm.at[c, :], wd.at[c, :], sems.at[SR + 2]),
        ]

    def after(x, t):
        if t is None:
            return x
        return x | jnp.tile(t, (x.shape[0] // 8, x.shape[1] // 128))

    def ln_rows(start, nrows, grp, paced, t=None):
        src = x_all.at[_ds(start, nrows, 16), :]
        dst = xn_all.at[_ds(start >> 1, nrows // 2, 8), :]
        if t is not None:
            x_all[S:S + 16, 0:128] = _unpack(t)
        cur = src[0:grp, :]
        ys = []
        for r in range(0, nrows, grp):
            xw = after(_pack(cur), t)
            y0, _ = _ln(_unpack2(xw, 0))
            y1, var = _ln(_unpack2(xw, 1))
            if r + grp < nrows:
                if paced:
                    e = jnp.broadcast_to(var[grp // 2 - 8:], (8, 128))
                    x_all[S:S + 16, 0:128] = _unpack(pltpu.bitcast(e, u32))
                cur = src[r + grp:r + 2 * grp, :]
            y = _pack2(y0, y1)
            dst[r // 2:(r + grp) // 2, :] = y
            ys.append(y)
            if paced:
                t = y[grp // 2 - 8:, D - 128:D] & zvec
        return ys

    def last_tok(u):
        return pltpu.bitcast(u[u.shape[0] - 8:, u.shape[1] - 128:], u32) & zvec

    def load_xn(start, nrows):
        return _unpack(xn_all[_ds(start >> 1, nrows // 2, 8), :])

    def scatter_rows(t, slot, m0):
        for m in range(t.shape[0] // DH):
            r = TB + (m0 + m) * PS
            wbuf[slot, r:r + DH, :] = t[m * DH:(m + 1) * DH, :]

    def gather_rows(slot, dst, t, mid=None):
        src = wbuf.at[slot + z]
        for d0 in range(0, DH, GD):
            y = jnp.concatenate(
                [src[pl.ds(TB + d, HH, stride=PS), :] for d in range(d0, d0 + GD)], axis=0)
            y = after(y, t)
            dst[d0 * HH:(d0 + GD) * HH, :] = y
            t = delay(y[GD * HH - 8:, :], DL) & zvec
            if mid is not None and d0 == DH // 2:
                mid(t)
        return t

    def load_w(r0):
        return _unpack(jnp.concatenate(
            [wbuf[c, r0:r0 + D // 2, :] for c in range(NC)], axis=1))

    def set_xn_cur(b, t):
        src = xn_all.at[_ds(b * (TM // 2), TM // 2, 8), :]
        if t is not None:
            xn_all[S // 2:S // 2 + 8, 0:128] = t
        for r in range(0, TM // 2, 8):
            y = after(src[r:r + 8, :], t)
            if t is not None:
                xn_all[S // 2:S // 2 + 8, 0:128] = y[:, 0:128]
                t = delay(y[:, D - 128:D], 2 * DL) & zvec
            xn_cur[r:r + 8, :] = y

    @pl.when(i == 0)
    @jax.named_scope('step0')
    def _step0():
        cp_x(0).start()
        cp_g(0).start()
        cp_u(0).start()
        cp_x(1).start()
        cp_d(0).start()
        for t in range(1, NSUB):
            cp_g(t).start()
            cp_u(t).start()
            cp_d(t).start()
            if t == 1:
                cp_x(2).start()
        for j in range(6):
            cp_q(j).start()
            if j < 4:
                cp_o(j).start()
            if 3 + j < NB:
                cp_x(3 + j).start()
        for c in cp_rest():
            c.start()

        abuf[0:2 * NC, TM:TM + HALO, :] = jnp.zeros((2 * NC, HALO, 128), f32)

        cp_x(0).wait()

        def lbody(r, c):
            ln_rows(r * 128, 128, 128, False)
            return c
        jax.lax.fori_loop(0, 2, lbody, 0)

        with jax.named_scope('s0a'):
            cp_g(0).wait()
            xn = load_xn(0, TM)
            g0 = _dot(xn, wg[:, 0:SUB])
            cp_u(0).wait()
            h0 = (_silu(g0) * _dot(xn, wu[:, 0:SUB])).astype(bf16)
            cp_x(1).wait()
            ys = ln_rows(TM, TM, 16, False)
            hs = [h0]
            for lo_r, hi_r in R3SPLIT:
                xn = _unpack(jnp.concatenate(ys[lo_r:hi_r], axis=0))
                g1 = _dot(xn, wg[:, 0:SUB])
                hs.append((_silu(g1) * _dot(xn, wu[:, 0:SUB])).astype(bf16))
            cp_d(0).wait()
            acc_all[0:2 * TM, :] = _dot(jnp.concatenate(hs, axis=0), wd[0:SUB, :])

        @jax.named_scope('s0body')
        def body(t, c):
            cols = _ds(t * SUB, SUB, SUB)
            cp_g(t).wait()
            cp_u(t).wait()
            cp_d(t).wait()

            @pl.when(t == 1)
            def _():
                cp_x(2).wait()
            xn = load_xn(0, 2 * TM)
            g = _dot(xn, wg[:, cols])
            u = _dot(xn, wu[:, cols])
            h = (_silu(g) * u).astype(bf16)
            acc_all[0:2 * TM, :] += _dot(h, wd[cols, :])
            ln_rows(2 * TM + (t - 1) * 128, 128, 32, True, last_tok(u))
            return c
        jax.lax.fori_loop(1, NSUB, body, 0)
        set_xn_cur(2, None)

    @pl.when(jnp.logical_and(i >= 1, i < N0))
    @jax.named_scope('phase0')
    def _phase0():
        b = i + 1
        j = i - 1
        cp_q(j).wait()

        @pl.when(j < 4)
        def _():
            cp_o(j).wait()

        @pl.when(b + 1 < NB)
        def _():
            cp_x(b + 1).wait()

        xn = _unpack(xn_cur[...])
        bn = jnp.minimum(b + 1, NB - 1)
        ln_rows(bn * TM, TM, 16, True)

        src = wqkv_raw.at[_ds((j & 1) * 512, 512, 512), _ds((j >> 1) * D, D, D)]
        drows = _ds((j >> 1) * (D // 2), D // 2, D // 2)
        jo = jnp.minimum(j, 3)
        osrc = wo_raw.at[:, _ds(jo * 256, 256, 256)]

        def gate_q(t):
            wqkv_raw[D:D + 16, 0:128] = _unpack(t)

        def gate_o(t):
            wo_raw[D:D + 16, 0:128] = _unpack(t)

        def ld_o(m0):
            return (osrc[m0 * DH:(m0 + 1) * DH, :], osrc[(m0 + HH) * DH:(m0 + HH + 1) * DH, :])

        t = None
        for n in range(4):
            lo = src[n * 128:(n + 1) * 128, 0:D // 2].astype(f32)
            hi = src[n * 128:(n + 1) * 128, D // 2:D].astype(f32)
            scatter_rows(_pack2(lo, hi).T, n, 0)
            t = gather_rows(n, wbuf.at[(j & 1) * 4 + n, drows], t, gate_q if n < 3 else gate_o)
        cur = ld_o(0)
        for m0 in range(HH):
            y = after(_pack2(cur[0].astype(f32), cur[1].astype(f32)), t)
            if m0 + 1 < HH:
                gate_o(y[0:8, 0:128])
                cur = ld_o(m0 + 1)
            scatter_rows(y[:, 0:128], 4, m0)
            scatter_rows(y[:, 128:256], 5, m0)
            t = delay(y[24:32, 128:256], 2 * DL) & zvec
        for n in range(2):
            t = gather_rows(4 + n, wbuf.at[jo * 2 + n, pl.ds(3 * D // 2, D // 2)], t)

        acc = None
        for lo_c, hi_c in P0CH:
            g = _dot(xn, wg[:, lo_c:hi_c])
            u = _dot(xn, wu[:, lo_c:hi_c])
            h = (_silu(g) * u).astype(bf16)
            d = _dot(h, wd[lo_c:hi_c, :])
            acc = d if acc is None else acc + d
        acc_all[_rows(b), :] = acc
        set_xn_cur(bn, last_tok(u))

    @pl.when(i >= N0)
    @jax.named_scope('phase1')
    def _phase1():
        b = i - N0

        @pl.when(i == N0)
        def _():
            for c in cp_rest():
                c.wait()

        @pl.when(b >= 2)
        def _():
            cp_out(b - 2).wait()

        abuf[0:2 * NC, 0:HALO, :] = abuf[0:2 * NC, TM:TM + HALO, :]

        xn = load_xn(b * TM, TM)

        def ffn(acc, lo_c, hi_c):
            g = _dot(xn, wg[:, lo_c:hi_c])
            u = _dot(xn, wu[:, lo_c:hi_c])
            h = (_silu(g) * u).astype(bf16)
            return acc + _dot(h, wd[lo_c:hi_c, :])

        acc = acc_all[_rows(b), :]
        for ch in FCH[:NPRE]:
            acc = ffn(acc, *ch)
        facc = acc
        for p, base in ((1, 0), (2, NC), (0, 2 * NC)):
            y = _dot_nt(xn, load_w(p * D // 2))
            for c in range(NC):
                abuf[base + c, HALO:HALO + TM, :] = y[:, c * 128:(c + 1) * 128]

        scale = DH ** -0.5

        ab = abuf.at[pl.ds(z, 3 * NC)]

        def tok(v):
            return pltpu.bitcast(pltpu.bitcast(v, u32) & zvec, f32)

        def gate(v):
            abuf[2 * NC, 0:RC, :] = v

        def ld_q(r0):
            return [ab[2 * NC + c, HALO + r0:HALO + r0 + RC, :] for c in range(NC)]

        def ld_k(r0, w):
            off = HALO + r0 - DIL * w
            return [ab[c, off:off + RC, :] for c in range(NC)]

        def ld_v(r0, c):
            return [ab[NC + c, HALO + r0 - DIL * w:HALO + r0 - DIL * w + RC, :] for w in range(W)]

        def chain(a, bs, prev, nxt):
            ts = [x * y for x, y in zip(a, bs)]
            acc = ts[0] if prev is None else ts[0] + tok(prev)
            res = None
            for n in range(1, 8):
                acc = acc + ts[n]
                if n == GPOS and nxt is not None:
                    gate(acc)
                    res = nxt()
            return acc, res

        prev = None
        q = ld_q(0)
        cur = ld_k(0, 0)
        for r0 in range(0, TM, RC):
            logits = []
            for w in range(W):
                nxt = (lambda: ld_k(r0, w + 1)) if w < W - 1 else None
                acc, cur = chain(q, cur, prev, nxt)
                prev = acc
                acc = acc + pltpu.roll(acc, 64, 1)
                acc = acc + pltpu.roll(acc, 32, 1)
                lg = acc * scale
                if r0 < DIL * w:
                    pos = b * TM + r0 + jax.lax.broadcasted_iota(jnp.int32, (RC, 128), 0)
                    lg = jnp.where(pos >= DIL * w, lg, -1e9)
                logits.append(lg)
            mx = functools.reduce(jnp.maximum, logits)
            gate(mx)
            cur = ld_v(r0, 0)
            ps = [jnp.exp(l - mx) for l in logits]
            den = functools.reduce(lambda a, b_: a + b_, ps)
            inv = pl.reciprocal(den, approx=True)
            inv = inv * (2.0 - den * inv)
            prev = None
            for c in range(NC):
                if c < NC - 1:
                    nxt = lambda: ld_v(r0, c + 1)
                elif r0 + RC < TM:
                    nxt = lambda: (ld_q(r0 + RC), ld_k(r0 + RC, 0))
                else:
                    nxt = None
                acc, cur = chain(ps, cur, prev, nxt)
                prev = acc
                abuf[2 * NC + c, HALO + r0:HALO + r0 + RC, :] = acc * inv
            if cur is not None:
                q, cur = cur

        acc = facc
        for ch in FCH[NPRE:]:
            acc = ffn(acc, *ch)

        o = jnp.concatenate(
            [abuf[2 * NC + c, HALO:HALO + TM, :].astype(bf16) for c in range(NC)], axis=1)
        s = _dot(o, load_w(3 * D // 2))
        ob = obuf.at[b & 1]
        for k in range(NOP):
            c = slice(k * OW, (k + 1) * OW)
            x = x_all[_rows(b), c].astype(f32)
            ob[:, c] = (x + s[:, c] * _silu(acc[:, c])).astype(bf16)
            cp_out(b, k).start()

        @pl.when(b == NB - 1)
        def _():
            cp_out(b - 1).wait()
            cp_out(b).wait()


@jax.jit
def pallas_recurrent_scan__sliding_local_dilated__swiglu_ffn__prompt_kernel(
    A_x, A_wqkv, A_wo, B_x, B_w_gate, B_w_up, B_w_down,
):
    x = A_x.reshape(S, D)
    out = pl.pallas_call(
        kernel,
        grid=(N0 + NB,),
        in_specs=[pl.BlockSpec(memory_space=pl.ANY)] * 6,
        out_specs=pl.BlockSpec(memory_space=pl.ANY),
        out_shape=jax.ShapeDtypeStruct((S, D), bf16),
        scratch_shapes=[
            pltpu.VMEM((S + PAD, D), bf16),
            pltpu.VMEM((S // 2 + 8, D), u32),
            pltpu.VMEM((S, D), f32),
            pltpu.VMEM((D + PAD, 3 * D), bf16),
            pltpu.VMEM((D + PAD, D), bf16),
            pltpu.VMEM((D, F), bf16),
            pltpu.VMEM((D, F), bf16),
            pltpu.VMEM((F, D), bf16),
            pltpu.VMEM((NC, TB + HH * PS + 16, 128), u32),
            pltpu.VMEM((3 * NC, TM + HALO, 128), f32),
            pltpu.VMEM((TM // 2, D), u32),
            pltpu.VMEM((2, TM, D), bf16),
            pltpu.SemaphoreType.DMA((NSEM,)),
        ],
        compiler_params=pltpu.CompilerParams(
            dimension_semantics=("arbitrary",), vmem_limit_bytes=100 * 2**20,
            disable_bounds_checks=True, disable_semaphore_checks=True),
    )(x, A_wqkv, A_wo, B_w_gate, B_w_up, B_w_down)
    return out.reshape(1, S, D)
```

```python
import functools

import jax
import jax.numpy as jnp
import jax.experimental.pallas as pl
import jax.experimental.pallas.tpu as pltpu

S, D, F = 2048, 1024, 3584
H, DH, W, DIL = 32, 32, 8, 2
EPS = 1e-5
TM = 256
NB = S // TM
N0 = NB - 1
TF0 = 768
SUB = 256
NSUB = TF0 // SUB
P0CH = ((0, 256), (256, 768))
FCH = ((3328, 3584), (768, 1280), (1280, 1792), (1792, 2304), (2304, 2816), (2816, 3328))
HALO = 16
RC = 8
NC = D // 128
HH = H // 2
PS = 33
TB = 2 * D
DL = 4
PAD = 16
NOP = 8
OW = D // NOP
f32, bf16, u32 = jnp.float32, jnp.bfloat16, jnp.uint32

SX, SG, SU, SD, SQ, SO, SR, SOUT, NSEM = 0, 8, 11, 14, 17, 23, 27, 30, 32


def _dot(a, b):
    return jnp.dot(a, b, preferred_element_type=f32)


def _dot_nt(a, b):
    return jax.lax.dot_general(a, b, (((1,), (1,)), ((), ())), preferred_element_type=f32)


def _silu(x):
    h = 0.5 * x
    return h + h * jnp.tanh(h)


def _bits(x):
    return jax.lax.bitcast_convert_type(x, u32)


def _f32(x):
    return jax.lax.bitcast_convert_type(x, f32)


def _pack2(lo, hi):
    return (_bits(lo.astype(f32)) >> 16) | _bits(hi.astype(f32))


def _unpack(x):
    return pltpu.bitcast(x, bf16)


def _ds(start, size, mult):
    if isinstance(start, int):
        return pl.ds(start, size)
    return pl.ds(pl.multiple_of(start, mult), size)


def _rows(b):
    return _ds(b * TM, TM, TM)


def _kernel(x_hbm, wqkv_hbm, wo_hbm, wg_hbm, wu_hbm, wd_hbm, o_hbm,
            x_all, xn_all, acc_all, wqkv_raw, wo_raw, wg, wu, wd,
            wbuf, abuf, obuf, sems):
    i = pl.program_id(0)
    z = jnp.minimum(i, 0)
    zvec = jnp.full((8, 128), z, jnp.int32).astype(u32)

    def cp_x(b):
        return pltpu.make_async_copy(x_hbm.at[_rows(b), :], x_all.at[_rows(b), :], sems.at[SX + b])

    def cp_g(t):
        c = _ds(t * SUB, SUB, SUB)
        return pltpu.make_async_copy(wg_hbm.at[:, c], wg.at[:, c], sems.at[SG + t])

    def cp_u(t):
        c = _ds(t * SUB, SUB, SUB)
        return pltpu.make_async_copy(wu_hbm.at[:, c], wu.at[:, c], sems.at[SU + t])

    def cp_d(t):
        c = _ds(t * SUB, SUB, SUB)
        return pltpu.make_async_copy(wd_hbm.at[c, :], wd.at[c, :], sems.at[SD + t])

    def cp_q(j):
        r = _ds((j & 1) * 512, 512, 512)
        c = _ds((j >> 1) * D, D, D)
        return pltpu.make_async_copy(wqkv_hbm.at[r, c], wqkv_raw.at[r, c], sems.at[SQ + j])

    def cp_o(j):
        c = _ds(j * 256, 256, 256)
        return pltpu.make_async_copy(wo_hbm.at[:, c], wo_raw.at[pl.ds(0, D), c], sems.at[SO + j])

    def cp_out(b, k=None):
        c = pl.ds(0, D) if k is None else pl.ds(k * OW, OW)
        return pltpu.make_async_copy(
            obuf.at[b & 1, :, c], o_hbm.at[_rows(b), c], sems.at[SOUT + (b & 1)])

    def cp_rest():
        c = pl.ds(TF0, F - TF0)
        return [
            pltpu.make_async_copy(wg_hbm.at[:, c], wg.at[:, c], sems.at[SR]),
            pltpu.make_async_copy(wu_hbm.at[:, c], wu.at[:, c], sems.at[SR + 1]),
            pltpu.make_async_copy(wd_hbm.at[c, :], wd.at[c, :], sems.at[SR + 2]),
        ]

    def delay(v, n):
        for k in range(n):
            v = (v + zvec) if k % 2 == 0 else (v ^ zvec)
        return v

    def after(x, t):
        if t is None:
            return x
        return x | jnp.tile(t, (x.shape[0] // 8, x.shape[1] // 128))

    def last_tok(u):
        return _bits(u[u.shape[0] - 8:, u.shape[1] - 128:]) & zvec

    def ln_rows(start, nrows, grp, paced, t=None):
        src = x_all.at[_ds(start, nrows, 16), :]
        dst = xn_all.at[_ds(start >> 1, nrows // 2, 8), :]
        if t is not None:
            x_all[S:S + 16, 0:128] = _unpack(t)
        cur = src[0:grp, :]
        ys = []
        for r in range(0, nrows, grp):
            x = cur.astype(f32)
            p = x[:, 0:128]
            if t is not None:
                p = p + jnp.tile(_f32(t), (grp // 8, 1))
            for c in range(1, NC):
                p = p + x[:, c * 128:(c + 1) * 128]
            xc = x - jnp.sum(p, axis=-1, keepdims=True) * (1.0 / D)
            var = jnp.sum(xc * xc, axis=-1, keepdims=True) * (1.0 / D)
            if r + grp < nrows:
                if paced:
                    e = jnp.broadcast_to(var[grp - 8:], (8, 128))
                    x_all[S:S + 16, 0:128] = _unpack(_bits(e))
                cur = src[r + grp:r + 2 * grp, :]
            y = xc * jax.lax.rsqrt(var + EPS)
            dst[r // 2:(r + grp) // 2, :] = pltpu.bitcast(y.astype(bf16), u32)
            ys.append(y)
            if paced:
                t = last_tok(y)
        return ys

    def load_xn(start, nrows):
        return _unpack(xn_all[_ds(start >> 1, nrows // 2, 8), :])

    def scatter_rows(t, slot, m0):
        for m in range(t.shape[0] // DH):
            r = TB + (m0 + m) * PS
            wbuf[slot, r:r + DH, :] = t[m * DH:(m + 1) * DH, :]

    def gather_rows(slot, dst, t, mid=None):
        src = wbuf.at[slot + z]
        for d in range(DH):
            y = after(src[pl.ds(TB + d, HH, stride=PS), :], t)
            dst[d * HH:(d + 1) * HH, :] = y
            t = delay(y[HH - 8:, :], DL) & zvec
            if mid is not None and d == DH // 2:
                mid(t)
        return t

    def load_w(r0):
        return _unpack(jnp.concatenate(
            [wbuf[c, r0:r0 + D // 2, :] for c in range(NC)], axis=1))

    @pl.when(i == 0)
    def _step0():
        cp_x(0).start()
        cp_g(0).start()
        cp_u(0).start()
        cp_x(1).start()
        cp_d(0).start()
        for t in range(1, NSUB):
            cp_g(t).start()
            cp_u(t).start()
            cp_d(t).start()
            if t == 1:
                cp_x(2).start()
        for j in range(6):
            cp_q(j).start()
            if j < 4:
                cp_o(j).start()
            if 3 + j < NB:
                cp_x(3 + j).start()
        for c in cp_rest():
            c.start()

        abuf[0:2 * NC, TM:TM + HALO, :] = jnp.zeros((2 * NC, HALO, 128), f32)

        cp_x(0).wait()

        def lbody(r, c):
            ln_rows(r * 128, 128, 128, False)
            return c
        jax.lax.fori_loop(0, 2, lbody, 0)

        cp_g(0).wait()
        xn = load_xn(0, TM)
        g0 = _dot(xn, wg[:, 0:SUB])
        cp_u(0).wait()
        hs = [(_silu(g0) * _dot(xn, wu[:, 0:SUB])).astype(bf16)]
        cp_x(1).wait()
        ys = ln_rows(TM, TM, 16, False)
        for lo_r, hi_r in ((0, 4), (4, 16)):
            xn = jnp.concatenate(ys[lo_r:hi_r], axis=0).astype(bf16)
            g1 = _dot(xn, wg[:, 0:SUB])
            hs.append((_silu(g1) * _dot(xn, wu[:, 0:SUB])).astype(bf16))
        cp_d(0).wait()
        acc_all[0:2 * TM, :] = _dot(jnp.concatenate(hs, axis=0), wd[0:SUB, :])

        def body(t, c):
            cols = _ds(t * SUB, SUB, SUB)
            cp_g(t).wait()
            cp_u(t).wait()
            cp_d(t).wait()

            @pl.when(t == 1)
            def _():
                cp_x(2).wait()
            xn = load_xn(0, 2 * TM)
            g = _dot(xn, wg[:, cols])
            u = _dot(xn, wu[:, cols])
            h = (_silu(g) * u).astype(bf16)
            acc_all[0:2 * TM, :] += _dot(h, wd[cols, :])
            ln_rows(2 * TM + (t - 1) * 128, 128, 32, True, last_tok(u))
            return c
        jax.lax.fori_loop(1, NSUB, body, 0)

    @pl.when(jnp.logical_and(i >= 1, i < N0))
    def _phase0():
        b = i + 1
        j = i - 1
        cp_q(j).wait()

        @pl.when(j < 4)
        def _():
            cp_o(j).wait()

        @pl.when(b + 1 < NB)
        def _():
            cp_x(b + 1).wait()

        xn = _unpack(after(xn_all[_ds(b * (TM // 2), TM // 2, 8), :], zvec))
        bn = jnp.minimum(b + 1, NB - 1)
        ln_rows(bn * TM, TM, 16, True)

        src = wqkv_raw.at[_ds((j & 1) * 512, 512, 512), _ds((j >> 1) * D, D, D)]
        drows = _ds((j >> 1) * (D // 2), D // 2, D // 2)
        jo = jnp.minimum(j, 3)
        osrc = wo_raw.at[:, _ds(jo * 256, 256, 256)]

        def gate_q(t):
            wqkv_raw[D:D + 16, 0:128] = _unpack(t)

        def gate_o(t):
            wo_raw[D:D + 16, 0:128] = _unpack(t)

        def ld_o(m0):
            return (osrc[m0 * DH:(m0 + 1) * DH, :], osrc[(m0 + HH) * DH:(m0 + HH + 1) * DH, :])

        t = None
        for n in range(4):
            lo = src[n * 128:(n + 1) * 128, 0:D // 2]
            hi = src[n * 128:(n + 1) * 128, D // 2:D]
            scatter_rows(_pack2(lo, hi).T, n, 0)
            t = gather_rows(n, wbuf.at[(j & 1) * 4 + n, drows], t, gate_q if n < 3 else gate_o)
        cur = ld_o(0)
        for m0 in range(HH):
            y = after(_pack2(*cur), t)
            if m0 + 1 < HH:
                gate_o(y[0:8, 0:128])
                cur = ld_o(m0 + 1)
            scatter_rows(y[:, 0:128], 4, m0)
            scatter_rows(y[:, 128:256], 5, m0)
            t = delay(y[24:32, 128:256], 2 * DL) & zvec
        for n in range(2):
            t = gather_rows(4 + n, wbuf.at[jo * 2 + n, pl.ds(3 * D // 2, D // 2)], t)

        acc = None
        for lo_c, hi_c in P0CH:
            g = _dot(xn, wg[:, lo_c:hi_c])
            u = _dot(xn, wu[:, lo_c:hi_c])
            h = (_silu(g) * u).astype(bf16)
            d = _dot(h, wd[lo_c:hi_c, :])
            acc = d if acc is None else acc + d
        acc_all[_rows(b), :] = acc

    @pl.when(i >= N0)
    def _phase1():
        b = i - N0

        @pl.when(i == N0)
        def _():
            for c in cp_rest():
                c.wait()

        @pl.when(b >= 2)
        def _():
            cp_out(b - 2).wait()

        abuf[0:2 * NC, 0:HALO, :] = abuf[0:2 * NC, TM:TM + HALO, :]

        xn = load_xn(b * TM, TM)

        def ffn(acc, lo_c, hi_c):
            g = _dot(xn, wg[:, lo_c:hi_c])
            u = _dot(xn, wu[:, lo_c:hi_c])
            h = (_silu(g) * u).astype(bf16)
            return acc + _dot(h, wd[lo_c:hi_c, :])

        facc = ffn(acc_all[_rows(b), :], *FCH[0])
        for p, base in ((1, 0), (2, NC), (0, 2 * NC)):
            y = _dot_nt(xn, load_w(p * D // 2))
            for c in range(NC):
                abuf[base + c, HALO:HALO + TM, :] = y[:, c * 128:(c + 1) * 128]

        ab = abuf.at[pl.ds(z, 3 * NC)]

        def gate(v):
            abuf[2 * NC, 0:RC, :] = v

        def ld_q(r0):
            return [ab[2 * NC + c, HALO + r0:HALO + r0 + RC, :] for c in range(NC)]

        def ld_k(r0, w):
            off = HALO + r0 - DIL * w
            return [ab[c, off:off + RC, :] for c in range(NC)]

        def ld_v(r0, c):
            return [ab[NC + c, HALO + r0 - DIL * w:HALO + r0 - DIL * w + RC, :] for w in range(W)]

        def chain(a, bs, prev, nxt):
            ts = [x * y for x, y in zip(a, bs)]
            acc = ts[0] if prev is None else ts[0] + _f32(_bits(prev) & zvec)
            acc = acc + ts[1]
            res = None
            if nxt is not None:
                gate(acc)
                res = nxt()
            for n in range(2, 8):
                acc = acc + ts[n]
            return acc, res

        prev = None
        q = ld_q(0)
        cur = ld_k(0, 0)
        for r0 in range(0, TM, RC):
            logits = []
            for w in range(W):
                nxt = (lambda: ld_k(r0, w + 1)) if w < W - 1 else None
                acc, cur = chain(q, cur, prev, nxt)
                prev = acc
                acc = acc + pltpu.roll(acc, 64, 1)
                acc = acc + pltpu.roll(acc, 32, 1)
                lg = acc * DH ** -0.5
                if r0 < DIL * w:
                    pos = b * TM + r0 + jax.lax.broadcasted_iota(jnp.int32, (RC, 128), 0)
                    lg = jnp.where(pos >= DIL * w, lg, -1e9)
                logits.append(lg)
            mx = functools.reduce(jnp.maximum, logits)
            gate(mx)
            cur = ld_v(r0, 0)
            ps = [jnp.exp(l - mx) for l in logits]
            den = functools.reduce(lambda u, v: u + v, ps)
            inv = pl.reciprocal(den, approx=True)
            inv = inv * (2.0 - den * inv)
            prev = None
            for c in range(NC):
                if c < NC - 1:
                    nxt = lambda: ld_v(r0, c + 1)
                elif r0 + RC < TM:
                    nxt = lambda: (ld_q(r0 + RC), ld_k(r0 + RC, 0))
                else:
                    nxt = None
                acc, cur = chain(ps, cur, prev, nxt)
                prev = acc
                abuf[2 * NC + c, HALO + r0:HALO + r0 + RC, :] = acc * inv
            if cur is not None:
                q, cur = cur

        for ch in FCH[1:]:
            facc = ffn(facc, *ch)

        o = jnp.concatenate(
            [abuf[2 * NC + c, HALO:HALO + TM, :].astype(bf16) for c in range(NC)], axis=1)
        s = _dot(o, load_w(3 * D // 2))
        ob = obuf.at[b & 1]
        for k in range(NOP):
            c = slice(k * OW, (k + 1) * OW)
            x = x_all[_rows(b), c].astype(f32)
            ob[:, c] = (x + s[:, c] * _silu(facc[:, c])).astype(bf16)
            cp_out(b, k).start()

        @pl.when(b == NB - 1)
        def _():
            cp_out(b - 1).wait()
            cp_out(b).wait()


@jax.jit
def pallas_recurrent_scan__sliding_local_dilated__swiglu_ffn__prompt_kernel(
    A_x: jax.Array,
    A_wqkv: jax.Array,
    A_wo: jax.Array,
    B_x: jax.Array,
    B_w_gate: jax.Array,
    B_w_up: jax.Array,
    B_w_down: jax.Array,
):
    out = pl.pallas_call(
        _kernel,
        grid=(N0 + NB,),
        in_specs=[pl.BlockSpec(memory_space=pl.ANY)] * 6,
        out_specs=pl.BlockSpec(memory_space=pl.ANY),
        out_shape=jax.ShapeDtypeStruct((S, D), bf16),
        scratch_shapes=[
            pltpu.VMEM((S + PAD, D), bf16),
            pltpu.VMEM((S // 2, D), u32),
            pltpu.VMEM((S, D), f32),
            pltpu.VMEM((D + PAD, 3 * D), bf16),
            pltpu.VMEM((D + PAD, D), bf16),
            pltpu.VMEM((D, F), bf16),
            pltpu.VMEM((D, F), bf16),
            pltpu.VMEM((F, D), bf16),
            pltpu.VMEM((NC, TB + HH * PS + 16, 128), u32),
            pltpu.VMEM((3 * NC, TM + HALO, 128), f32),
            pltpu.VMEM((2, TM, D), bf16),
            pltpu.SemaphoreType.DMA((NSEM,)),
        ],
        compiler_params=pltpu.CompilerParams(
            dimension_semantics=("arbitrary",), vmem_limit_bytes=100 * 2**20,
            disable_bounds_checks=True, disable_semaphore_checks=True),
    )(A_x.reshape(S, D), A_wqkv, A_wo, B_w_gate, B_w_up, B_w_down)
    return out.reshape(1, S, D)
```

```python
import functools

import jax
import jax.numpy as jnp
import jax.experimental.pallas as pl
import jax.experimental.pallas.tpu as pltpu

S, D, F = 2048, 1024, 3584
H, DH, W, DIL = 32, 32, 8, 2
EPS = 1e-5
TM = 256
NB = S // TM
TF0 = 768
SUB = 256
NSUB = TF0 // SUB
P0CH = ((0, 256), (256, 768))
FCH = ((3328, 3584), (768, 1280), (1280, 1792), (1792, 2304), (2304, 2816), (2816, 3328))
HALO = 16
RC = 8
NC = D // 128
HH = H // 2
PS = 33
TB = 2 * D
DL = 4
PAD = 16
NOP = 8
OW = D // NOP
f32, bf16, u32 = jnp.float32, jnp.bfloat16, jnp.uint32

SX, SG, SU, SD, SQ, SO, SR, SOUT, NSEM = 0, 8, 11, 14, 17, 23, 27, 30, 31


def _dot(a, b):
    return jnp.dot(a, b, preferred_element_type=f32)


def _dot_nt(a, b):
    return jax.lax.dot_general(a, b, (((1,), (1,)), ((), ())), preferred_element_type=f32)


def _silu(x):
    h = 0.5 * x
    return h + h * jnp.tanh(h)


def _bits(x):
    return jax.lax.bitcast_convert_type(x, u32)


def _f32(x):
    return jax.lax.bitcast_convert_type(x, f32)


def _pack2(lo, hi):
    return (_bits(lo.astype(f32)) >> 16) | _bits(hi.astype(f32))


def _unpack(x):
    return pltpu.bitcast(x, bf16)


def _ds(start, size, mult):
    if isinstance(start, int):
        return pl.ds(start, size)
    return pl.ds(pl.multiple_of(start, mult), size)


def _rows(b):
    return _ds(b * TM, TM, TM)


def _kernel(x_hbm, wqkv_hbm, wo_hbm, wg_hbm, wu_hbm, wd_hbm, o_hbm,
            x_all, xn_all, acc_all, wqkv_raw, wo_raw, wg, wu, wd,
            wbuf, abuf, obuf, sems):
    zero = {}

    def set_zero(idx):
        zero['s'] = jnp.minimum(idx, 0)
        zero['v'] = jnp.full((8, 128), zero['s'], jnp.int32).astype(u32)

    def cp_x(b):
        return pltpu.make_async_copy(x_hbm.at[_rows(b), :], x_all.at[_rows(b), :], sems.at[SX + b])

    def cp_g(t):
        c = _ds(t * SUB, SUB, SUB)
        return pltpu.make_async_copy(wg_hbm.at[:, c], wg.at[:, c], sems.at[SG + t])

    def cp_u(t):
        c = _ds(t * SUB, SUB, SUB)
        return pltpu.make_async_copy(wu_hbm.at[:, c], wu.at[:, c], sems.at[SU + t])

    def cp_d(t):
        c = _ds(t * SUB, SUB, SUB)
        return pltpu.make_async_copy(wd_hbm.at[c, :], wd.at[c, :], sems.at[SD + t])

    def cp_q(j):
        r = _ds((j & 1) * 512, 512, 512)
        c = _ds((j >> 1) * D, D, D)
        return pltpu.make_async_copy(wqkv_hbm.at[r, c], wqkv_raw.at[r, c], sems.at[SQ + j])

    def cp_o(j):
        c = _ds(j * 256, 256, 256)
        return pltpu.make_async_copy(wo_hbm.at[:, c], wo_raw.at[pl.ds(0, D), c], sems.at[SO + j])

    def cp_out(b, k):
        c = pl.ds(k * OW, OW)
        return pltpu.make_async_copy(obuf.at[_rows(b), c], o_hbm.at[_rows(b), c], sems.at[SOUT])

    def cp_rest():
        c = pl.ds(TF0, F - TF0)
        return [
            pltpu.make_async_copy(wg_hbm.at[:, c], wg.at[:, c], sems.at[SR]),
            pltpu.make_async_copy(wu_hbm.at[:, c], wu.at[:, c], sems.at[SR + 1]),
            pltpu.make_async_copy(wd_hbm.at[c, :], wd.at[c, :], sems.at[SR + 2]),
        ]

    def delay(v, n):
        for k in range(n):
            v = (v + zero['v']) if k % 2 == 0 else (v ^ zero['v'])
        return v

    def after(x, t):
        if t is None:
            return x
        return x | jnp.tile(t, (x.shape[0] // 8, x.shape[1] // 128))

    def last_tok(u):
        return _bits(u[u.shape[0] - 8:, u.shape[1] - 128:]) & zero['v']

    def ln_rows(start, nrows, grp, paced, t=None):
        src = x_all.at[_ds(start, nrows, 16), :]
        dst = xn_all.at[_ds(start >> 1, nrows // 2, 8), :]
        if t is not None:
            x_all[S:S + 16, 0:128] = _unpack(t)
        cur = src[0:grp, :]
        ys = []
        for r in range(0, nrows, grp):
            x = cur.astype(f32)
            p = x[:, 0:128]
            if t is not None:
                p = p + jnp.tile(_f32(t), (grp // 8, 1))
            for c in range(1, NC):
                p = p + x[:, c * 128:(c + 1) * 128]
            xc = x - jnp.sum(p, axis=-1, keepdims=True) * (1.0 / D)
            var = jnp.sum(xc * xc, axis=-1, keepdims=True) * (1.0 / D)
            if r + grp < nrows:
                if paced:
                    e = jnp.broadcast_to(var[grp - 8:], (8, 128))
                    x_all[S:S + 16, 0:128] = _unpack(_bits(e))
                cur = src[r + grp:r + 2 * grp, :]
            y = xc * jax.lax.rsqrt(var + EPS)
            dst[r // 2:(r + grp) // 2, :] = pltpu.bitcast(y.astype(bf16), u32)
            ys.append(y)
            if paced:
                t = last_tok(y)
        return ys

    def load_xn(start, nrows):
        return _unpack(xn_all[_ds(start >> 1, nrows // 2, 8), :])

    def scatter_rows(t, slot, m0):
        for m in range(t.shape[0] // DH):
            r = TB + (m0 + m) * PS
            wbuf[slot, r:r + DH, :] = t[m * DH:(m + 1) * DH, :]

    def gather_rows(slot, dst, t, mid=None):
        src = wbuf.at[slot + zero['s']]
        for d in range(DH):
            y = after(src[pl.ds(TB + d, HH, stride=PS), :], t)
            dst[d * HH:(d + 1) * HH, :] = y
            t = delay(y[HH - 8:, :], DL) & zero['v']
            if mid is not None and d == DH // 2:
                mid(t)
        return t

    def load_w(r0):
        return _unpack(jnp.concatenate(
            [wbuf[c, r0:r0 + D // 2, :] for c in range(NC)], axis=1))

    def _step0():
        cp_x(0).start()
        cp_g(0).start()
        cp_u(0).start()
        cp_x(1).start()
        cp_d(0).start()
        for t in range(1, NSUB):
            cp_g(t).start()
            cp_u(t).start()
            cp_d(t).start()
            if t == 1:
                cp_x(2).start()
        for j in range(6):
            cp_q(j).start()
            if j < 4:
                cp_o(j).start()
            if 3 + j < NB:
                cp_x(3 + j).start()
        for c in cp_rest():
            c.start()

        abuf[0:2 * NC, TM:TM + HALO, :] = jnp.zeros((2 * NC, HALO, 128), f32)

        cp_x(0).wait()

        def lbody(r, c):
            ln_rows(r * 128, 128, 128, False)
            return c
        jax.lax.fori_loop(0, 2, lbody, 0)

        cp_g(0).wait()
        xn = load_xn(0, TM)
        g0 = _dot(xn, wg[:, 0:SUB])
        cp_u(0).wait()
        hs = [(_silu(g0) * _dot(xn, wu[:, 0:SUB])).astype(bf16)]
        cp_x(1).wait()
        ys = ln_rows(TM, TM, 16, False)
        for lo_r, hi_r in ((0, 4), (4, 16)):
            xn = jnp.concatenate(ys[lo_r:hi_r], axis=0).astype(bf16)
            g1 = _dot(xn, wg[:, 0:SUB])
            hs.append((_silu(g1) * _dot(xn, wu[:, 0:SUB])).astype(bf16))
        cp_d(0).wait()
        acc_all[0:2 * TM, :] = _dot(jnp.concatenate(hs, axis=0), wd[0:SUB, :])

        def body(t, c):
            set_zero(t)
            cols = _ds(t * SUB, SUB, SUB)
            cp_g(t).wait()
            cp_u(t).wait()
            cp_d(t).wait()

            @pl.when(t == 1)
            def _():
                cp_x(2).wait()
            xn = load_xn(0, 2 * TM)
            g = _dot(xn, wg[:, cols])
            u = _dot(xn, wu[:, cols])
            h = (_silu(g) * u).astype(bf16)
            acc_all[0:2 * TM, :] += _dot(h, wd[cols, :])
            ln_rows(2 * TM + (t - 1) * 128, 128, 32, True, last_tok(u))
            return c
        jax.lax.fori_loop(1, NSUB, body, 0)

    def _phase0(i, carry):
        set_zero(i)
        b = i + 1
        j = i - 1
        cp_q(j).wait()

        @pl.when(j < 4)
        def _():
            cp_o(j).wait()

        @pl.when(b + 1 < NB)
        def _():
            cp_x(b + 1).wait()

        xn = _unpack(after(xn_all[_ds(b * (TM // 2), TM // 2, 8), :], zero['v']))
        bn = jnp.minimum(b + 1, NB - 1)
        ln_rows(bn * TM, TM, 16, True)

        src = wqkv_raw.at[_ds((j & 1) * 512, 512, 512), _ds((j >> 1) * D, D, D)]
        drows = _ds((j >> 1) * (D // 2), D // 2, D // 2)
        jo = jnp.minimum(j, 3)
        osrc = wo_raw.at[:, _ds(jo * 256, 256, 256)]

        def gate_q(t):
            wqkv_raw[D:D + 16, 0:128] = _unpack(t)

        def gate_o(t):
            wo_raw[D:D + 16, 0:128] = _unpack(t)

        def ld_o(m0):
            return (osrc[m0 * DH:(m0 + 1) * DH, :], osrc[(m0 + HH) * DH:(m0 + HH + 1) * DH, :])

        t = None
        for n in range(4):
            lo = src[n * 128:(n + 1) * 128, 0:D // 2]
            hi = src[n * 128:(n + 1) * 128, D // 2:D]
            scatter_rows(_pack2(lo, hi).T, n, 0)
            t = gather_rows(n, wbuf.at[(j & 1) * 4 + n, drows], t, gate_q if n < 3 else gate_o)
        cur = ld_o(0)
        for m0 in range(HH):
            y = after(_pack2(*cur), t)
            if m0 + 1 < HH:
                gate_o(y[0:8, 0:128])
                cur = ld_o(m0 + 1)
            scatter_rows(y[:, 0:128], 4, m0)
            scatter_rows(y[:, 128:256], 5, m0)
            t = delay(y[24:32, 128:256], 2 * DL) & zero['v']
        for n in range(2):
            t = gather_rows(4 + n, wbuf.at[jo * 2 + n, pl.ds(3 * D // 2, D // 2)], t)

        acc = None
        for lo_c, hi_c in P0CH:
            g = _dot(xn, wg[:, lo_c:hi_c])
            u = _dot(xn, wu[:, lo_c:hi_c])
            h = (_silu(g) * u).astype(bf16)
            d = _dot(h, wd[lo_c:hi_c, :])
            acc = d if acc is None else acc + d
        acc_all[_rows(b), :] = acc
        return carry

    def _phase1(b, carry):
        set_zero(b)

        abuf[0:2 * NC, 0:HALO, :] = abuf[0:2 * NC, TM:TM + HALO, :]

        xn = load_xn(b * TM, TM)

        def ffn(acc, lo_c, hi_c):
            g = _dot(xn, wg[:, lo_c:hi_c])
            u = _dot(xn, wu[:, lo_c:hi_c])
            h = (_silu(g) * u).astype(bf16)
            return acc + _dot(h, wd[lo_c:hi_c, :])

        facc = ffn(acc_all[_rows(b), :], *FCH[0])
        for p, base in ((1, 0), (2, NC), (0, 2 * NC)):
            y = _dot_nt(xn, load_w(p * D // 2))
            for c in range(NC):
                abuf[base + c, HALO:HALO + TM, :] = y[:, c * 128:(c + 1) * 128]

        ab = abuf.at[pl.ds(zero['s'], 3 * NC)]

        def gate(v):
            abuf[2 * NC, 0:RC, :] = v

        def ld_q(r0):
            return [ab[2 * NC + c, HALO + r0:HALO + r0 + RC, :] for c in range(NC)]

        def ld_k(r0, w):
            off = HALO + r0 - DIL * w
            return [ab[c, off:off + RC, :] for c in range(NC)]

        def ld_v(r0, c):
            return [ab[NC + c, HALO + r0 - DIL * w:HALO + r0 - DIL * w + RC, :] for w in range(W)]

        def chain(a, bs, prev, nxt):
            ts = [x * y for x, y in zip(a, bs)]
            acc = ts[0] if prev is None else ts[0] + _f32(_bits(prev) & zero['v'])
            acc = acc + ts[1]
            res = None
            if nxt is not None:
                gate(acc)
                res = nxt()
            for n in range(2, 8):
                acc = acc + ts[n]
            return acc, res

        prev = None
        q = ld_q(0)
        cur = ld_k(0, 0)
        for r0 in range(0, TM, RC):
            logits = []
            for w in range(W):
                nxt = (lambda: ld_k(r0, w + 1)) if w < W - 1 else None
                acc, cur = chain(q, cur, prev, nxt)
                prev = acc
                acc = acc + pltpu.roll(acc, 64, 1)
                acc = acc + pltpu.roll(acc, 32, 1)
                lg = acc * DH ** -0.5
                if r0 < DIL * w:
                    pos = b * TM + r0 + jax.lax.broadcasted_iota(jnp.int32, (RC, 128), 0)
                    lg = jnp.where(pos >= DIL * w, lg, -1e9)
                logits.append(lg)
            mx = functools.reduce(jnp.maximum, logits)
            gate(mx)
            cur = ld_v(r0, 0)
            ps = [jnp.exp(l - mx) for l in logits]
            den = functools.reduce(lambda u, v: u + v, ps)
            inv = pl.reciprocal(den, approx=True)
            inv = inv * (2.0 - den * inv)
            prev = None
            for c in range(NC):
                if c < NC - 1:
                    nxt = lambda: ld_v(r0, c + 1)
                elif r0 + RC < TM:
                    nxt = lambda: (ld_q(r0 + RC), ld_k(r0 + RC, 0))
                else:
                    nxt = None
                acc, cur = chain(ps, cur, prev, nxt)
                prev = acc
                abuf[2 * NC + c, HALO + r0:HALO + r0 + RC, :] = acc * inv
            if cur is not None:
                q, cur = cur

        for ch in FCH[1:]:
            facc = ffn(facc, *ch)

        o = jnp.concatenate(
            [abuf[2 * NC + c, HALO:HALO + TM, :].astype(bf16) for c in range(NC)], axis=1)
        s = _dot(o, load_w(3 * D // 2))
        ob = obuf.at[_rows(b)]
        for k in range(NOP):
            c = slice(k * OW, (k + 1) * OW)
            x = x_all[_rows(b), c].astype(f32)
            ob[:, c] = (x + s[:, c] * _silu(facc[:, c])).astype(bf16)
            cp_out(b, k).start()

        return carry

    _step0()
    jax.lax.fori_loop(1, NB - 1, _phase0, 0)
    for c in cp_rest():
        c.wait()
    jax.lax.fori_loop(0, NB, _phase1, 0)
    pltpu.make_async_copy(obuf, o_hbm, sems.at[SOUT]).wait()


@jax.jit
def pallas_recurrent_scan__sliding_local_dilated__swiglu_ffn__prompt_kernel(
    A_x: jax.Array,
    A_wqkv: jax.Array,
    A_wo: jax.Array,
    B_x: jax.Array,
    B_w_gate: jax.Array,
    B_w_up: jax.Array,
    B_w_down: jax.Array,
):
    out = pl.pallas_call(
        _kernel,
        in_specs=[pl.BlockSpec(memory_space=pl.ANY)] * 6,
        out_specs=pl.BlockSpec(memory_space=pl.ANY),
        out_shape=jax.ShapeDtypeStruct((S, D), bf16),
        scratch_shapes=[
            pltpu.VMEM((S + PAD, D), bf16),
            pltpu.VMEM((S // 2, D), u32),
            pltpu.VMEM((S, D), f32),
            pltpu.VMEM((D + PAD, 3 * D), bf16),
            pltpu.VMEM((D + PAD, D), bf16),
            pltpu.VMEM((D, F), bf16),
            pltpu.VMEM((D, F), bf16),
            pltpu.VMEM((F, D), bf16),
            pltpu.VMEM((NC, TB + HH * PS + 16, 128), u32),
            pltpu.VMEM((3 * NC, TM + HALO, 128), f32),
            pltpu.VMEM((S, D), bf16),
            pltpu.SemaphoreType.DMA((NSEM,)),
        ],
        compiler_params=pltpu.CompilerParams(
            vmem_limit_bytes=100 * 2**20,
            disable_bounds_checks=True, disable_semaphore_checks=True),
    )(A_x.reshape(S, D), A_wqkv, A_wo, B_w_gate, B_w_up, B_w_down)
    return out.reshape(1, S, D)
```

```python
import functools

import jax
import jax.numpy as jnp
import jax.experimental.pallas as pl
import jax.experimental.pallas.tpu as pltpu

S, D, F = 2048, 1024, 3584
H, DH, W, DIL = 32, 32, 8, 2
EPS = 1e-5
TM = 256
NB = S // TM
TF0 = 768
SUB = 256
NSUB = TF0 // SUB
P0CH = ((0, 768),)
FCH = ((3328, 3584), (768, 1280), (1280, 1792), (1792, 2304), (2304, 2816), (2816, 3328))
HALO = 16
RC = 8
NC = D // 128
HH = H // 2
PS = 33
TB = 2 * D
DL = 3
PAD = 16
NOP = 8
OW = D // NOP
f32, bf16, u32 = jnp.float32, jnp.bfloat16, jnp.uint32

SX, SG, SU, SD, SQ, SO, SR, SOUT, NSEM = 0, 8, 11, 14, 17, 23, 27, 30, 31


def _dot(a, b):
    return jnp.dot(a, b, preferred_element_type=f32)


def _dot_nt(a, b):
    return jax.lax.dot_general(a, b, (((1,), (1,)), ((), ())), preferred_element_type=f32)


def _silu(x):
    h = 0.5 * x
    return h + h * jnp.tanh(h)


def _bits(x):
    return jax.lax.bitcast_convert_type(x, u32)


def _f32(x):
    return jax.lax.bitcast_convert_type(x, f32)


def _pack2(lo, hi):
    return (_bits(lo.astype(f32)) >> 16) | _bits(hi.astype(f32))


def _unpack(x):
    return pltpu.bitcast(x, bf16)


def _ds(start, size, mult):
    if isinstance(start, int):
        return pl.ds(start, size)
    return pl.ds(pl.multiple_of(start, mult), size)


def _rows(b):
    return _ds(b * TM, TM, TM)


def _kernel(x_hbm, wqkv_hbm, wo_hbm, wg_hbm, wu_hbm, wd_hbm, o_hbm,
            x_all, xn_all, acc_all, wqkv_raw, wo_raw, wg, wu, wd,
            wbuf, abuf, obuf, sems):
    zero = {}

    def set_zero(idx):
        zero['s'] = jnp.minimum(idx, 0)
        zero['v'] = jnp.full((8, 128), zero['s'], jnp.int32).astype(u32)

    def cp_x(b):
        return pltpu.make_async_copy(x_hbm.at[_rows(b), :], x_all.at[_rows(b), :], sems.at[SX + b])

    def cp_g(t):
        c = _ds(t * SUB, SUB, SUB)
        return pltpu.make_async_copy(wg_hbm.at[:, c], wg.at[:, c], sems.at[SG + t])

    def cp_u(t):
        c = _ds(t * SUB, SUB, SUB)
        return pltpu.make_async_copy(wu_hbm.at[:, c], wu.at[:, c], sems.at[SU + t])

    def cp_d(t):
        c = _ds(t * SUB, SUB, SUB)
        return pltpu.make_async_copy(wd_hbm.at[c, :], wd.at[c, :], sems.at[SD + t])

    def cp_q(j):
        r = _ds((j & 1) * 512, 512, 512)
        c = _ds((j >> 1) * D, D, D)
        return pltpu.make_async_copy(wqkv_hbm.at[r, c], wqkv_raw.at[r, c], sems.at[SQ + j])

    def cp_o(j):
        c = _ds(j * 256, 256, 256)
        return pltpu.make_async_copy(wo_hbm.at[:, c], wo_raw.at[pl.ds(0, D), c], sems.at[SO + j])

    def cp_out(b, k):
        c = pl.ds(k * OW, OW)
        return pltpu.make_async_copy(obuf.at[_rows(b), c], o_hbm.at[_rows(b), c], sems.at[SOUT])

    def cp_rest():
        c = pl.ds(TF0, F - TF0)
        return [
            pltpu.make_async_copy(wg_hbm.at[:, c], wg.at[:, c], sems.at[SR]),
            pltpu.make_async_copy(wu_hbm.at[:, c], wu.at[:, c], sems.at[SR + 1]),
            pltpu.make_async_copy(wd_hbm.at[c, :], wd.at[c, :], sems.at[SR + 2]),
        ]

    def delay(v, n):
        for k in range(n):
            v = (v + zero['v']) if k % 2 == 0 else (v ^ zero['v'])
        return v

    def after(x, t):
        if t is None:
            return x
        return x | jnp.tile(t, (x.shape[0] // 8, x.shape[1] // 128))

    def last_tok(u):
        return _bits(u[u.shape[0] - 8:, u.shape[1] - 128:]) & zero['v']

    def ln_rows(start, nrows, grp, paced, t=None):
        src = x_all.at[_ds(start, nrows, 16), :]
        dst = xn_all.at[_ds(start >> 1, nrows // 2, 8), :]
        if t is not None:
            x_all[S:S + 16, 0:128] = _unpack(t)
        cur = src[0:grp, :]
        ys = []
        for r in range(0, nrows, grp):
            x = cur.astype(f32)
            p = x[:, 0:128]
            if t is not None:
                p = p + jnp.tile(_f32(t), (grp // 8, 1))
            for c in range(1, NC):
                p = p + x[:, c * 128:(c + 1) * 128]
            xc = x - jnp.sum(p, axis=-1, keepdims=True) * (1.0 / D)
            var = jnp.sum(xc * xc, axis=-1, keepdims=True) * (1.0 / D)
            if r + grp < nrows:
                if paced:
                    e = jnp.broadcast_to(var[grp - 16:grp - 8], (8, 128))
                    x_all[S:S + 16, 0:128] = _unpack(_bits(e))
                cur = src[r + grp:r + 2 * grp, :]
            y = xc * jax.lax.rsqrt(var + EPS)
            dst[r // 2:(r + grp) // 2, :] = pltpu.bitcast(y.astype(bf16), u32)
            ys.append(y)
            if paced:
                t = last_tok(y[0:y.shape[0] - 8])
        return ys

    def load_xn(start, nrows):
        return _unpack(xn_all[_ds(start >> 1, nrows // 2, 8), :])

    def scatter_rows(t, slot, m0):
        for m in range(t.shape[0] // DH):
            r = TB + (m0 + m) * PS
            wbuf[slot, r:r + DH, :] = t[m * DH:(m + 1) * DH, :]

    def gather_rows(slot, dst, t, mid=None):
        src = wbuf.at[slot + zero['s']]
        for d in range(DH):
            y = after(src[pl.ds(TB + d, HH, stride=PS), :], t)
            dst[d * HH:(d + 1) * HH, :] = y
            t = delay(y[HH - 8:, :], DL) & zero['v']
            if mid is not None and d == 10:
                mid(t)
        return t

    def load_w(r0):
        return _unpack(jnp.concatenate(
            [wbuf[c, r0:r0 + D // 2, :] for c in range(NC)], axis=1))

    def _step0():
        cp_x(0).start()
        cp_g(0).start()
        cp_u(0).start()
        cp_x(1).start()
        cp_d(0).start()
        for t in range(1, NSUB):
            cp_g(t).start()
            cp_u(t).start()
            cp_d(t).start()
            if t == 1:
                cp_x(2).start()
        for j in range(6):
            cp_q(j).start()
            if j < 4:
                cp_o(j).start()
            if 3 + j < NB:
                cp_x(3 + j).start()
        for c in cp_rest():
            c.start()

        abuf[0:2 * NC, TM:TM + HALO, :] = jnp.zeros((2 * NC, HALO, 128), f32)

        cp_x(0).wait()

        def lbody(r, c):
            ln_rows(r * 128, 128, 128, False)
            return c
        jax.lax.fori_loop(0, 2, lbody, 0)

        cp_g(0).wait()
        xn = load_xn(0, TM)
        g0 = _dot(xn, wg[:, 0:SUB])
        cp_u(0).wait()
        hs = [(_silu(g0) * _dot(xn, wu[:, 0:SUB])).astype(bf16)]
        cp_x(1).wait()
        ys = ln_rows(TM, TM, 16, False)
        for lo_r, hi_r in ((0, 4), (4, 16)):
            xn = jnp.concatenate(ys[lo_r:hi_r], axis=0).astype(bf16)
            g1 = _dot(xn, wg[:, 0:SUB])
            hs.append((_silu(g1) * _dot(xn, wu[:, 0:SUB])).astype(bf16))
        cp_d(0).wait()
        acc_all[0:2 * TM, :] = _dot(jnp.concatenate(hs, axis=0), wd[0:SUB, :])

        def body(t, c):
            set_zero(t)
            cols = _ds(t * SUB, SUB, SUB)
            cp_g(t).wait()
            cp_u(t).wait()
            cp_d(t).wait()

            @pl.when(t == 1)
            def _():
                cp_x(2).wait()
            xn = load_xn(0, 2 * TM)
            g = _dot(xn, wg[:, cols])
            u = _dot(xn, wu[:, cols])
            h = (_silu(g) * u).astype(bf16)
            acc_all[0:2 * TM, :] += _dot(h, wd[cols, :])
            ln_rows(2 * TM + (t - 1) * 128, 128, 32, True, last_tok(u))
            return c
        jax.lax.fori_loop(1, NSUB, body, 0)

    def _phase0(i, carry):
        set_zero(i)
        b = i + 1
        j = i - 1
        cp_q(j).wait()

        @pl.when(j < 4)
        def _():
            cp_o(j).wait()

        @pl.when(b + 1 < NB)
        def _():
            cp_x(b + 1).wait()

        xn = _unpack(after(xn_all[_ds(b * (TM // 2), TM // 2, 8), :], zero['v']))
        bn = jnp.minimum(b + 1, NB - 1)
        ln_rows(bn * TM, TM, 16, True)

        src = wqkv_raw.at[_ds((j & 1) * 512, 512, 512), _ds((j >> 1) * D, D, D)]
        drows = _ds((j >> 1) * (D // 2), D // 2, D // 2)
        jo = jnp.minimum(j, 3)
        osrc = wo_raw.at[:, _ds(jo * 256, 256, 256)]

        def gate_q(t):
            wqkv_raw[D:D + 16, 0:128] = _unpack(t)

        def gate_o(t):
            wo_raw[D:D + 16, 0:128] = _unpack(t)

        def ld_o(m0):
            return (osrc[m0 * DH:(m0 + 1) * DH, :], osrc[(m0 + HH) * DH:(m0 + HH + 1) * DH, :])

        t = None
        for n in range(4):
            lo = src[n * 128:(n + 1) * 128, 0:D // 2]
            hi = src[n * 128:(n + 1) * 128, D // 2:D]
            scatter_rows(_pack2(lo, hi).T, n, 0)
            t = gather_rows(n, wbuf.at[(j & 1) * 4 + n, drows], t, gate_q if n < 3 else gate_o)
        cur = ld_o(0)
        for m0 in range(HH):
            y = after(_pack2(*cur), t)
            if m0 + 1 < HH:
                gate_o(y[0:8, 0:128])
                cur = ld_o(m0 + 1)
            scatter_rows(y[:, 0:128], 4, m0)
            scatter_rows(y[:, 128:256], 5, m0)
            t = delay(y[24:32, 128:256], 4 * DL) & zero['v']
        for n in range(2):
            t = gather_rows(4 + n, wbuf.at[jo * 2 + n, pl.ds(3 * D // 2, D // 2)], t)

        acc = None
        for lo_c, hi_c in P0CH:
            g = _dot(xn, wg[:, lo_c:hi_c])
            u = _dot(xn, wu[:, lo_c:hi_c])
            h = (_silu(g) * u).astype(bf16)
            d = _dot(h, wd[lo_c:hi_c, :])
            acc = d if acc is None else acc + d
        acc_all[_rows(b), :] = acc
        return carry

    def _phase1(b, carry):
        set_zero(b)

        abuf[0:2 * NC, 0:HALO, :] = abuf[0:2 * NC, TM:TM + HALO, :]

        xn = load_xn(b * TM, TM)

        def ffn(acc, lo_c, hi_c):
            g = _dot(xn, wg[:, lo_c:hi_c])
            u = _dot(xn, wu[:, lo_c:hi_c])
            h = (_silu(g) * u).astype(bf16)
            return acc + _dot(h, wd[lo_c:hi_c, :])

        facc = ffn(acc_all[_rows(b), :], *FCH[0])
        for p, base in ((1, 0), (2, NC), (0, 2 * NC)):
            y = _dot_nt(xn, load_w(p * D // 2))
            for c in range(NC):
                abuf[base + c, HALO:HALO + TM, :] = y[:, c * 128:(c + 1) * 128]

        ab = abuf.at[pl.ds(zero['s'], 3 * NC)]

        def gate(v):
            abuf[2 * NC, 0:RC, :] = v

        def ld_q(r0):
            return [ab[2 * NC + c, HALO + r0:HALO + r0 + RC, :] for c in range(NC)]

        def ld_k(r0, w):
            off = HALO + r0 - DIL * w
            return [ab[c, off:off + RC, :] for c in range(NC)]

        def ld_v(r0, c):
            return [ab[NC + c, HALO + r0 - DIL * w:HALO + r0 - DIL * w + RC, :] for w in range(W)]

        def chain(a, bs, prev, nxt):
            ts = [x * y for x, y in zip(a, bs)]
            acc = ts[0] if prev is None else ts[0] + _f32(_bits(prev) & zero['v'])
            acc = acc + ts[1]
            res = None
            if nxt is not None:
                gate(acc)
                res = nxt()
            for n in range(2, 8):
                acc = acc + ts[n]
            return acc, res

        prev = None
        q = ld_q(0)
        cur = ld_k(0, 0)
        for r0 in range(0, TM, RC):
            logits = []
            for w in range(W):
                nxt = (lambda: ld_k(r0, w + 1)) if w < W - 1 else None
                acc, cur = chain(q, cur, prev, nxt)
                prev = acc
                acc = acc + pltpu.roll(acc, 64, 1)
                acc = acc + pltpu.roll(acc, 32, 1)
                lg = acc * DH ** -0.5
                if r0 < DIL * w:
                    pos = b * TM + r0 + jax.lax.broadcasted_iota(jnp.int32, (RC, 128), 0)
                    lg = jnp.where(pos >= DIL * w, lg, -1e9)
                logits.append(lg)
            mx = functools.reduce(jnp.maximum, logits)
            gate(mx)
            cur = ld_v(r0, 0)
            ps = [jnp.exp(l - mx) for l in logits]
            den = functools.reduce(lambda u, v: u + v, ps)
            inv = pl.reciprocal(den, approx=True)
            inv = inv * (2.0 - den * inv)
            prev = None
            for c in range(NC):
                if c < NC - 1:
                    nxt = lambda: ld_v(r0, c + 1)
                elif r0 + RC < TM:
                    nxt = lambda: (ld_q(r0 + RC), ld_k(r0 + RC, 0))
                else:
                    nxt = None
                acc, cur = chain(ps, cur, prev, nxt)
                prev = acc
                abuf[2 * NC + c, HALO + r0:HALO + r0 + RC, :] = acc * inv
            if cur is not None:
                q, cur = cur

        for ch in FCH[1:]:
            facc = ffn(facc, *ch)

        o = jnp.concatenate(
            [abuf[2 * NC + c, HALO:HALO + TM, :].astype(bf16) for c in range(NC)], axis=1)
        s = _dot(o, load_w(3 * D // 2))
        ob = obuf.at[_rows(b)]
        for k in range(NOP):
            c = slice(k * OW, (k + 1) * OW)
            x = x_all[_rows(b), c].astype(f32)
            ob[:, c] = (x + s[:, c] * _silu(facc[:, c])).astype(bf16)
            cp_out(b, k).start()

        return carry

    _step0()
    jax.lax.fori_loop(1, NB - 1, _phase0, 0)
    for c in cp_rest():
        c.wait()
    jax.lax.fori_loop(0, NB, _phase1, 0)
    pltpu.make_async_copy(obuf, o_hbm, sems.at[SOUT]).wait()


@jax.jit
def pallas_recurrent_scan__sliding_local_dilated__swiglu_ffn__prompt_kernel(
    A_x: jax.Array,
    A_wqkv: jax.Array,
    A_wo: jax.Array,
    B_x: jax.Array,
    B_w_gate: jax.Array,
    B_w_up: jax.Array,
    B_w_down: jax.Array,
):
    out = pl.pallas_call(
        _kernel,
        in_specs=[pl.BlockSpec(memory_space=pl.ANY)] * 6,
        out_specs=pl.BlockSpec(memory_space=pl.ANY),
        out_shape=jax.ShapeDtypeStruct((S, D), bf16),
        scratch_shapes=[
            pltpu.VMEM((S + PAD, D), bf16),
            pltpu.VMEM((S // 2, D), u32),
            pltpu.VMEM((S, D), f32),
            pltpu.VMEM((D + PAD, 3 * D), bf16),
            pltpu.VMEM((D + PAD, D), bf16),
            pltpu.VMEM((D, F), bf16),
            pltpu.VMEM((D, F), bf16),
            pltpu.VMEM((F, D), bf16),
            pltpu.VMEM((NC, TB + HH * PS + 16, 128), u32),
            pltpu.VMEM((3 * NC, TM + HALO, 128), f32),
            pltpu.VMEM((S, D), bf16),
            pltpu.SemaphoreType.DMA((NSEM,)),
        ],
        compiler_params=pltpu.CompilerParams(
            vmem_limit_bytes=100 * 2**20,
            disable_bounds_checks=True, disable_semaphore_checks=True),
    )(A_x.reshape(S, D), A_wqkv, A_wo, B_w_gate, B_w_up, B_w_down)
    return out.reshape(1, S, D)
```

```python
import functools

import jax
import jax.numpy as jnp
import jax.experimental.pallas as pl
import jax.experimental.pallas.tpu as pltpu

S, D, F = 2048, 1024, 3584
H, DH, W, DIL = 32, 32, 8, 2
EPS = 1e-5
TM = 256
NB = S // TM
TF0 = 768
SUB = 256
NSUB = TF0 // SUB
P0CH = ((0, 768),)
FCH = ((3328, 3584), (768, 1280), (1280, 1792), (1792, 2304), (2304, 2816), (2816, 3328))
HALO = 16
RC = 8
NC = D // 128
HH = H // 2
PS = 33
TB = 2 * D
DL = 3
PAD = 16
NOP = 8
OW = D // NOP
f32, bf16, u32 = jnp.float32, jnp.bfloat16, jnp.uint32

SX, SG, SU, SD, SQ, SO, SR, SOUT, SX2, NSEM = 0, 8, 11, 14, 17, 23, 27, 30, 31, 33


def _dot(a, b):
    return jnp.dot(a, b, preferred_element_type=f32)


def _dot_nt(a, b):
    return jax.lax.dot_general(a, b, (((1,), (1,)), ((), ())), preferred_element_type=f32)


def _silu(x):
    h = 0.5 * x
    return h + h * jnp.tanh(h)


def _bits(x):
    return jax.lax.bitcast_convert_type(x, u32)


def _f32(x):
    return jax.lax.bitcast_convert_type(x, f32)


def _pack2(lo, hi):
    return (_bits(lo.astype(f32)) >> 16) | _bits(hi.astype(f32))


def _unpack(x):
    return pltpu.bitcast(x, bf16)


def _ds(start, size, mult):
    if isinstance(start, int):
        return pl.ds(start, size)
    return pl.ds(pl.multiple_of(start, mult), size)


def _rows(b):
    return _ds(b * TM, TM, TM)


def _kernel(x_hbm, wqkv_hbm, wo_hbm, wg_hbm, wu_hbm, wd_hbm, o_hbm,
            x_all, xn_all, acc_all, wqkv_raw, wo_raw, wg, wu, wd,
            wbuf, abuf, obuf, sems):
    zero = {}

    def set_zero(idx):
        zero['s'] = jnp.minimum(idx, 0)
        zero['v'] = jnp.full((8, 128), zero['s'], jnp.int32).astype(u32)

    def cp_x(b):
        return pltpu.make_async_copy(x_hbm.at[_rows(b), :], x_all.at[_rows(b), :], sems.at[SX + b])

    def cp_x2(k):
        r = _ds(2 * TM + k * (TM // 2), TM // 2, TM // 2)
        return pltpu.make_async_copy(x_hbm.at[r, :], x_all.at[r, :], sems.at[SX2 + k])

    def cp_g(t):
        c = _ds(t * SUB, SUB, SUB)
        return pltpu.make_async_copy(wg_hbm.at[:, c], wg.at[:, c], sems.at[SG + t])

    def cp_u(t):
        c = _ds(t * SUB, SUB, SUB)
        return pltpu.make_async_copy(wu_hbm.at[:, c], wu.at[:, c], sems.at[SU + t])

    def cp_d(t):
        c = _ds(t * SUB, SUB, SUB)
        return pltpu.make_async_copy(wd_hbm.at[c, :], wd.at[c, :], sems.at[SD + t])

    def cp_q(j):
        r = _ds((j & 1) * 512, 512, 512)
        c = _ds((j >> 1) * D, D, D)
        return pltpu.make_async_copy(wqkv_hbm.at[r, c], wqkv_raw.at[r, c], sems.at[SQ + j])

    def cp_o(j):
        c = _ds(j * 256, 256, 256)
        return pltpu.make_async_copy(wo_hbm.at[:, c], wo_raw.at[pl.ds(0, D), c], sems.at[SO + j])

    def cp_out(b, k):
        c = pl.ds(k * OW, OW)
        return pltpu.make_async_copy(obuf.at[_rows(b), c], o_hbm.at[_rows(b), c], sems.at[SOUT])

    def cp_rest():
        c = pl.ds(TF0, F - TF0)
        return [
            pltpu.make_async_copy(wg_hbm.at[:, c], wg.at[:, c], sems.at[SR]),
            pltpu.make_async_copy(wu_hbm.at[:, c], wu.at[:, c], sems.at[SR + 1]),
            pltpu.make_async_copy(wd_hbm.at[c, :], wd.at[c, :], sems.at[SR + 2]),
        ]

    def delay(v, n):
        for k in range(n):
            v = (v + zero['v']) if k % 2 == 0 else (v ^ zero['v'])
        return v

    def after(x, t):
        if t is None:
            return x
        return x | jnp.tile(t, (x.shape[0] // 8, x.shape[1] // 128))

    def last_tok(u):
        return _bits(u[u.shape[0] - 8:, u.shape[1] - 128:]) & zero['v']

    def ln_rows(start, nrows, grp, paced, t=None):
        src = x_all.at[_ds(start, nrows, 16), :]
        dst = xn_all.at[_ds(start >> 1, nrows // 2, 8), :]
        if t is not None:
            x_all[S:S + 16, 0:128] = _unpack(t)
        cur = src[0:grp, :]
        ys = []
        for r in range(0, nrows, grp):
            x = cur.astype(f32)
            p = x[:, 0:128]
            if t is not None:
                p = p + jnp.tile(_f32(t), (grp // 8, 1))
            for c in range(1, NC):
                p = p + x[:, c * 128:(c + 1) * 128]
            xc = x - jnp.sum(p, axis=-1, keepdims=True) * (1.0 / D)
            var = jnp.sum(xc * xc, axis=-1, keepdims=True) * (1.0 / D)
            if r + grp < nrows:
                if paced:
                    e = jnp.broadcast_to(var[grp - 16:grp - 8], (8, 128))
                    x_all[S:S + 16, 0:128] = _unpack(_bits(e))
                cur = src[r + grp:r + 2 * grp, :]
            y = xc * jax.lax.rsqrt(var + EPS)
            dst[r // 2:(r + grp) // 2, :] = pltpu.bitcast(y.astype(bf16), u32)
            ys.append(y)
            if paced:
                t = last_tok(y[0:y.shape[0] - 8])
        return ys

    def load_xn(start, nrows):
        return _unpack(xn_all[_ds(start >> 1, nrows // 2, 8), :])

    def scatter_rows(t, slot, m0):
        for m in range(t.shape[0] // DH):
            r = TB + (m0 + m) * PS
            wbuf[slot, r:r + DH, :] = t[m * DH:(m + 1) * DH, :]

    def gather_rows(slot, dst, t, mid=None):
        src = wbuf.at[slot + zero['s']]
        for d in range(DH):
            y = after(src[pl.ds(TB + d, HH, stride=PS), :], t)
            dst[d * HH:(d + 1) * HH, :] = y
            t = delay(y[HH - 8:, :], DL) & zero['v']
            if mid is not None and d == 10:
                mid(t)
        return t

    def load_w(r0):
        return _unpack(jnp.concatenate(
            [wbuf[c, r0:r0 + D // 2, :] for c in range(NC)], axis=1))

    def _step0():
        cp_x(0).start()
        cp_g(0).start()
        cp_u(0).start()
        cp_x(1).start()
        cp_d(0).start()
        for t in range(1, NSUB):
            cp_g(t).start()
            cp_u(t).start()
            cp_d(t).start()
            cp_x2(t - 1).start()
        for j in range(6):
            cp_q(j).start()
            if j < 4:
                cp_o(j).start()
            if 3 + j < NB:
                cp_x(3 + j).start()
        for c in cp_rest():
            c.start()

        abuf[0:2 * NC, TM:TM + HALO, :] = jnp.zeros((2 * NC, HALO, 128), f32)

        cp_x(0).wait()

        def lbody(r, c):
            ln_rows(r * 128, 128, 128, False)
            return c
        jax.lax.fori_loop(0, 2, lbody, 0)

        cp_g(0).wait()
        xn = load_xn(0, TM)
        g0 = _dot(xn, wg[:, 0:SUB])
        cp_u(0).wait()
        hs = [(_silu(g0[0:192]) * _dot(xn[0:192], wu[:, 0:SUB])).astype(bf16)]
        cp_x(1).wait()
        hs.append((_silu(g0[192:TM]) * _dot(xn[192:TM], wu[:, 0:SUB])).astype(bf16))
        ys = ln_rows(TM, TM, 16, False)
        for lo_r, hi_r in ((0, 4), (4, 16)):
            xn = jnp.concatenate(ys[lo_r:hi_r], axis=0).astype(bf16)
            g1 = _dot(xn, wg[:, 0:SUB])
            hs.append((_silu(g1) * _dot(xn, wu[:, 0:SUB])).astype(bf16))
        cp_d(0).wait()
        acc_all[0:2 * TM, :] = _dot(jnp.concatenate(hs, axis=0), wd[0:SUB, :])

        def body(t, c):
            set_zero(t)
            cols = _ds(t * SUB, SUB, SUB)
            cp_g(t).wait()
            cp_u(t).wait()
            cp_d(t).wait()
            cp_x2(t - 1).wait()
            xn = load_xn(0, 2 * TM)
            g = _dot(xn, wg[:, cols])
            u = _dot(xn, wu[:, cols])
            h = (_silu(g) * u).astype(bf16)
            acc_all[0:2 * TM, :] += _dot(h, wd[cols, :])
            ln_rows(2 * TM + (t - 1) * 128, 128, 32, True, last_tok(u))
            return c
        jax.lax.fori_loop(1, NSUB, body, 0)

    def _phase0(i, carry):
        set_zero(i)
        b = i + 1
        j = i - 1
        cp_q(j).wait()

        @pl.when(j < 4)
        def _():
            cp_o(j).wait()

        @pl.when(b + 1 < NB)
        def _():
            cp_x(b + 1).wait()

        xn = _unpack(after(xn_all[_ds(b * (TM // 2), TM // 2, 8), :], zero['v']))
        bn = jnp.minimum(b + 1, NB - 1)
        ln_rows(bn * TM, TM, 16, True)

        src = wqkv_raw.at[_ds((j & 1) * 512, 512, 512), _ds((j >> 1) * D, D, D)]
        drows = _ds((j >> 1) * (D // 2), D // 2, D // 2)
        jo = jnp.minimum(j, 3)
        osrc = wo_raw.at[:, _ds(jo * 256, 256, 256)]

        def gate_q(t):
            wqkv_raw[D:D + 16, 0:128] = _unpack(t)

        def gate_o(t):
            wo_raw[D:D + 16, 0:128] = _unpack(t)

        def ld_o(m0):
            return (osrc[m0 * DH:(m0 + 1) * DH, :], osrc[(m0 + HH) * DH:(m0 + HH + 1) * DH, :])

        t = None
        for n in range(4):
            lo = src[n * 128:(n + 1) * 128, 0:D // 2]
            hi = src[n * 128:(n + 1) * 128, D // 2:D]
            scatter_rows(_pack2(lo, hi).T, n, 0)
            t = gather_rows(n, wbuf.at[(j & 1) * 4 + n, drows], t, gate_q if n < 3 else gate_o)
        cur = ld_o(0)
        for m0 in range(HH):
            y = after(_pack2(*cur), t)
            if m0 + 1 < HH:
                gate_o(y[0:8, 0:128])
                cur = ld_o(m0 + 1)
            scatter_rows(y[:, 0:128], 4, m0)
            scatter_rows(y[:, 128:256], 5, m0)
            t = delay(y[24:32, 128:256], 4 * DL) & zero['v']
        for n in range(2):
            t = gather_rows(4 + n, wbuf.at[jo * 2 + n, pl.ds(3 * D // 2, D // 2)], t)

        acc = None
        for lo_c, hi_c in P0CH:
            g = _dot(xn, wg[:, lo_c:hi_c])
            u = _dot(xn, wu[:, lo_c:hi_c])
            h = (_silu(g) * u).astype(bf16)
            d = _dot(h, wd[lo_c:hi_c, :])
            acc = d if acc is None else acc + d
        acc_all[_rows(b), :] = acc
        return carry

    def _phase1(b, carry):
        set_zero(b)

        abuf[0:2 * NC, 0:HALO, :] = abuf[0:2 * NC, TM:TM + HALO, :]

        xn = load_xn(b * TM, TM)

        def ffn(acc, lo_c, hi_c):
            g = _dot(xn, wg[:, lo_c:hi_c])
            u = _dot(xn, wu[:, lo_c:hi_c])
            h = (_silu(g) * u).astype(bf16)
            return acc + _dot(h, wd[lo_c:hi_c, :])

        facc = ffn(acc_all[_rows(b), :], *FCH[0])
        for p, base in ((1, 0), (2, NC), (0, 2 * NC)):
            y = _dot_nt(xn, load_w(p * D // 2))
            for c in range(NC):
                abuf[base + c, HALO:HALO + TM, :] = y[:, c * 128:(c + 1) * 128]

        ab = abuf.at[pl.ds(zero['s'], 3 * NC)]

        def gate(v):
            abuf[2 * NC, 0:RC, :] = v

        def ld_q(r0):
            return [ab[2 * NC + c, HALO + r0:HALO + r0 + RC, :] for c in range(NC)]

        def ld_k(r0, w):
            off = HALO + r0 - DIL * w
            return [ab[c, off:off + RC, :] for c in range(NC)]

        def ld_v(r0, c):
            return [ab[NC + c, HALO + r0 - DIL * w:HALO + r0 - DIL * w + RC, :] for w in range(W)]

        def chain(a, bs, prev, nxt):
            ts = [x * y for x, y in zip(a, bs)]
            acc = ts[0] if prev is None else ts[0] + _f32(_bits(prev) & zero['v'])
            acc = acc + ts[1]
            res = None
            if nxt is not None:
                gate(acc)
                res = nxt()
            for n in range(2, 8):
                acc = acc + ts[n]
            return acc, res

        prev = None
        q = ld_q(0)
        cur = ld_k(0, 0)
        for r0 in range(0, TM, RC):
            logits = []
            for w in range(W):
                nxt = (lambda: ld_k(r0, w + 1)) if w < W - 1 else None
                acc, cur = chain(q, cur, prev, nxt)
                prev = acc
                acc = acc + pltpu.roll(acc, 64, 1)
                acc = acc + pltpu.roll(acc, 32, 1)
                lg = acc * DH ** -0.5
                if r0 < DIL * w:
                    pos = b * TM + r0 + jax.lax.broadcasted_iota(jnp.int32, (RC, 128), 0)
                    lg = jnp.where(pos >= DIL * w, lg, -1e9)
                logits.append(lg)
            mx = functools.reduce(jnp.maximum, logits)
            gate(mx)
            cur = ld_v(r0, 0)
            ps = [jnp.exp(l - mx) for l in logits]
            den = functools.reduce(lambda u, v: u + v, ps)
            inv = pl.reciprocal(den, approx=True)
            inv = inv * (2.0 - den * inv)
            prev = None
            for c in range(NC):
                if c < NC - 1:
                    nxt = lambda: ld_v(r0, c + 1)
                elif r0 + RC < TM:
                    nxt = lambda: (ld_q(r0 + RC), ld_k(r0 + RC, 0))
                else:
                    nxt = None
                acc, cur = chain(ps, cur, prev, nxt)
                prev = acc
                abuf[2 * NC + c, HALO + r0:HALO + r0 + RC, :] = acc * inv
            if cur is not None:
                q, cur = cur

        for ch in FCH[1:]:
            facc = ffn(facc, *ch)

        o = jnp.concatenate(
            [abuf[2 * NC + c, HALO:HALO + TM, :].astype(bf16) for c in range(NC)], axis=1)
        s = _dot(o, load_w(3 * D // 2))
        ob = obuf.at[_rows(b)]
        for k in range(NOP):
            c = slice(k * OW, (k + 1) * OW)
            x = x_all[_rows(b), c].astype(f32)
            ob[:, c] = (x + s[:, c] * _silu(facc[:, c])).astype(bf16)
            cp_out(b, k).start()

        return carry

    _step0()
    jax.lax.fori_loop(1, NB - 1, _phase0, 0)
    for c in cp_rest():
        c.wait()
    jax.lax.fori_loop(0, NB, _phase1, 0)
    pltpu.make_async_copy(obuf, o_hbm, sems.at[SOUT]).wait()


@jax.jit
def pallas_recurrent_scan__sliding_local_dilated__swiglu_ffn__prompt_kernel(
    A_x: jax.Array,
    A_wqkv: jax.Array,
    A_wo: jax.Array,
    B_x: jax.Array,
    B_w_gate: jax.Array,
    B_w_up: jax.Array,
    B_w_down: jax.Array,
):
    out = pl.pallas_call(
        _kernel,
        in_specs=[pl.BlockSpec(memory_space=pl.ANY)] * 6,
        out_specs=pl.BlockSpec(memory_space=pl.ANY),
        out_shape=jax.ShapeDtypeStruct((S, D), bf16),
        scratch_shapes=[
            pltpu.VMEM((S + PAD, D), bf16),
            pltpu.VMEM((S // 2, D), u32),
            pltpu.VMEM((S, D), f32),
            pltpu.VMEM((D + PAD, 3 * D), bf16),
            pltpu.VMEM((D + PAD, D), bf16),
            pltpu.VMEM((D, F), bf16),
            pltpu.VMEM((D, F), bf16),
            pltpu.VMEM((F, D), bf16),
            pltpu.VMEM((NC, TB + HH * PS + 16, 128), u32),
            pltpu.VMEM((3 * NC, TM + HALO, 128), f32),
            pltpu.VMEM((S, D), bf16),
            pltpu.SemaphoreType.DMA((NSEM,)),
        ],
        compiler_params=pltpu.CompilerParams(
            vmem_limit_bytes=100 * 2**20,
            disable_bounds_checks=True, disable_semaphore_checks=True),
    )(A_x.reshape(S, D), A_wqkv, A_wo, B_w_gate, B_w_up, B_w_down)
    return out.reshape(1, S, D)
```
